```python
import os as _os
_os.environ.setdefault("JAX_PLATFORMS", "cpu")
import jax
import jax.numpy as jnp

def _softmax(x, axis=-1):
    return jax.nn.softmax(x, axis=axis)
def _gelu(x):
    return jax.nn.gelu(x, approximate=True)
def _silu(x):
    return jax.nn.silu(x)
def _sigmoid(x):
    return jax.nn.sigmoid(x)
def _layernorm(x, axis=-1, eps=1e-5):
    m = jnp.mean(x, axis=axis, keepdims=True)
    v = jnp.var(x, axis=axis, keepdims=True)
    return (x - m) / jnp.sqrt(v + eps)
def _scatter_add(tgt, idx, src, axis=0):
    return tgt.at[idx].add(src)
def _segment_sum(src, seg, n):
    return jax.ops.segment_sum(src, seg, n)
class _Rng:
    def __init__(self, key):
        self._k = key
    def _next(self):
        self._k, sub = jax.random.split(self._k)
        return sub
    def normal(self, shape):
        return jax.random.normal(self._next(), shape, dtype=jnp.bfloat16)
    def randint(self, lo, hi, shape):
        return jax.random.randint(self._next(), shape, lo, hi, dtype=jnp.int32)
    def uniform(self, shape, lo=0.0, hi=1.0):
        return jax.random.uniform(self._next(), shape, jnp.bfloat16, lo, hi)
    def permutation(self, n):
        return jax.random.permutation(self._next(), n)


kernel_name = 'concat_heads__sliding_block__ssm_conv_s4__prompt'

def setup_inputs():
    _rng = _Rng(jax.random.key(int.from_bytes(__import__("os").urandom(4), "little")))
    _w = (lambda a: (lambda t: t.astype(jnp.bfloat16) if jnp.issubdtype(t.dtype, jnp.floating) else t)(jnp.asarray(a)))
    def _A_setup():
        B, S, D = 1, 2048, 512
        return {
            "x": _w((lambda *s: _rng.normal(s) * 0.2)(B, S, D)),
            "wqkv": _w((lambda *s: _rng.normal(s) * 0.2)(D, 3 * D)),
            "wo": _w((lambda *s: _rng.normal(s) * 0.05)(D, D)),
        }
    _A_in = _A_setup()

    def _B_setup():
        B, L, D, N = 1, 2048, 512, 128
        A_re = -jnp.exp((lambda *s: _rng.normal(s) * 0.8)(D, N))
        A_im = jnp.pi * (lambda *s: _rng.normal(s) * 0.8)(D, N)
        B_re = (lambda *s: _rng.normal(s) * 0.8)(D, N)
        B_im = (lambda *s: _rng.normal(s) * 0.8)(D, N)
        C_re = (lambda *s: _rng.normal(s) * 0.8)(D, N)
        C_im = (lambda *s: _rng.normal(s) * 0.8)(D, N)
        log_dt = (lambda *s: _rng.normal(s) * 0.8)(D) * 0.5 - 4.0
        Dskip = (lambda *s: _rng.normal(s) * 0.05)(D)
        return {
            "u": _w((lambda *s: _rng.normal(s) * 0.05)(B, L, D)),
            "A_re": _w(A_re),
            "A_im": _w(A_im),
            "B_re": _w(B_re),
            "B_im": _w(B_im),
            "C_re": _w(C_re),
            "C_im": _w(C_im),
            "log_dt": _w(log_dt),
            "Dskip": _w(Dskip),
        }
    _B_in = _B_setup()

    return {
        "A_x": _A_in["x"],
        "A_wqkv": _A_in["wqkv"],
        "A_wo": _A_in["wo"],
        "B_u": _B_in["u"],
        "B_A_re": _B_in["A_re"],
        "B_A_im": _B_in["A_im"],
        "B_B_re": _B_in["B_re"],
        "B_B_im": _B_in["B_im"],
        "B_C_re": _B_in["C_re"],
        "B_C_im": _B_in["C_im"],
        "B_log_dt": _B_in["log_dt"],
        "B_Dskip": _B_in["Dskip"],
    }

def reference(A_x, A_wqkv, A_wo, B_u, B_A_re, B_A_im, B_B_re, B_B_im, B_C_re, B_C_im, B_log_dt, B_Dskip):
    def _A_ref(x, wqkv, wo):
        B, S, D = x.shape
        H = 32; Dh = D // H; W = 256
        qkv = (lambda x, *d: x.transpose(*d))((x @ wqkv).reshape(B, S, 3, H, Dh), 2, 0, 3, 1, 4)
        q, k, v = qkv[0], qkv[1], qkv[2]
        scores = jnp.einsum("bhqd,bhkd->bhqk", q, k) * (Dh ** -0.5)
        idx = jnp.arange(S)
        mask = (idx[:, None] - idx[None, :] >= 0) & (idx[:, None] - idx[None, :] < W)
        scores = jnp.where(mask[None, None], scores, -1e9)
        p = _softmax(scores, axis=-1)
        o = jnp.einsum("bhqk,bhkd->bhqd", p, v)
        return (lambda x, *d: x.transpose(*d))(o, 0, 2, 1, 3).reshape(B, S, D) @ wo

    def _B_ref(u, A_re, A_im, B_re, B_im, C_re, C_im, log_dt, Dskip):
        Bsz, L, D = u.shape
        dt = jnp.exp(log_dt)[:, None]
        A = A_re + 1j * A_im
        Bc = B_re + 1j * B_im
        Cc = C_re + 1j * C_im
        logdA = dt * A
        dB = dt * Bc
        l = (lambda x, dt: x.astype(dt))(jnp.arange(L), A_re.dtype)
        P = jnp.exp(logdA[:, :, None] * l[None, None, :])
        K = jnp.einsum("dn,dnl,dn->dl", Cc, P, dB).real
        L2 = 2 * L
        Kp = jnp.pad(K, ((0, 0), (0, L)))
        up = (lambda x, *d: x.transpose(*d))(u, 0, 2, 1)
        up = jnp.pad(up, ((0, 0), (0, 0), (0, L)))
        Kf = (lambda x, axes=(-2,-1): jnp.fft.rfft2(x.astype(jnp.float32), axes=axes))(Kp[:, None, :], axes=(-2, -1))
        Uf = (lambda x, axes=(-2,-1): jnp.fft.rfft2(x.astype(jnp.float32), axes=axes))(up[:, :, None, :], axes=(-2, -1))
        Yf = Uf * Kf[None, :, :, :]
        y = (lambda x, s, axes=(-2,-1): jnp.fft.irfft2(x, s=s, axes=axes).astype(jnp.bfloat16))(Yf, (1, L2), axes=(-2, -1))[:, :, 0, :L]
        y = (lambda x, *d: x.transpose(*d))(y, 0, 2, 1) + u * Dskip[None, None, :]
        return y

    a = _A_ref(A_x, A_wqkv, A_wo)
    b = _B_ref(B_u, B_A_re, B_A_im, B_B_re, B_B_im, B_C_re, B_C_im, B_log_dt, B_Dskip)
    return jnp.concatenate([a, b], axis=-1)
```

```python
import functools

import jax
import jax.numpy as jnp
import ml_dtypes
import numpy as np
from jax import lax
from jax.experimental import pallas as pl
from jax.experimental.pallas import tpu as pltpu

S, D, H, DH, W = 2048, 512, 32, 16, 256
BQ = 128
NQ = S // BQ
L, N, T = 2048, 128, 128
NC = L // T
f32, bf16 = jnp.float32, jnp.bfloat16


def _split_hi_lo(m):
    hi = m.astype(np.float32).astype(ml_dtypes.bfloat16)
    lo = (m - hi.astype(np.float64)).astype(np.float32).astype(ml_dtypes.bfloat16)
    return hi, lo


def _dft_tables():
    f = np.arange(T)[:, None]
    j = np.arange(T)[None, :]
    th = 2 * np.pi * (f + 0.5) * j / (2 * T)
    F1 = np.concatenate([np.cos(th), -np.sin(th)], 0)
    tabs = []
    for reg, sigma in enumerate([1, 2, 4, 8]):
        base = 0 if reg == 0 else T * sigma
        m = base + np.arange(T)
        r = m.astype(np.float32).astype(ml_dtypes.bfloat16).astype(np.float64)
        idx = np.round((r - base) / sigma).astype(np.int64)
        Fp = np.zeros((2 * T, T))
        for jj in range(T):
            Fp[:, idx[jj]] += F1[:, jj]
        hi, lo = _split_hi_lo(Fp)
        tabs.append(np.concatenate([hi, lo], 0))
    Ftab = np.stack(tabs, 0)
    t = (np.arange(T) + T)[:, None]
    f2 = np.arange(T)[None, :]
    th2 = 2 * np.pi * (f2 + 0.5) * t / (2 * T)
    IF = np.concatenate([np.cos(th2), -np.sin(th2)], 1) / T
    hi, lo = _split_hi_lo(IF)
    IFtab = np.concatenate([hi, lo], 0)
    return Ftab, IFtab


def _cmul(ar, ai, br, bi):
    return ar * br - ai * bi, ar * bi + ai * br


def _dot(a, b):
    return jnp.dot(a, b, preferred_element_type=f32)


def _nt(a, b):
    return lax.dot_general(a, b, (((1,), (1,)), ((), ())), preferred_element_type=f32)


def _kernel(x_ref, wqT_ref, wk_ref, wvT_ref, wo_ref,
            u_ref, p_ref, ldt_ref, dsk_ref, F_ref, IF_ref,
            o_ref,
            kc_s, vc_s, qm_s, bias_s, ot_s, sa_s, sb_s,
            a_s, c_s, pw_s, lo_s, g_s, kq_s, uh_s, kp_s, ap_s, y_s):
    i = pl.program_id(0)

    @pl.when(i == 0)
    def _init():
        kc_s[:, 0:256, :] = jnp.zeros((4, 256, 128), bf16)
        vc_s[0:2] = jnp.zeros((2, D, BQ), bf16)
        qm_s[...] = jnp.zeros(qm_s.shape, bf16)

    x = x_ref[...]
    k = _dot(x, wk_ref[...]).astype(bf16)
    row0 = pl.multiple_of((i + 2) * BQ, BQ)
    for g in range(4):
        kc_s[g, pl.ds(row0, BQ), :] = k[:, g * 128:(g + 1) * 128]
    qT = (_nt(wqT_ref[...], x).astype(bf16) * 0.25).astype(bf16)
    for h in range(H):
        hp = h % 8
        qm_s[h // 8, hp * 16:hp * 16 + 16, hp * 128:(hp + 1) * 128] = qT[h * 16:(h + 1) * 16, :]
    vc_s[i + 2] = _nt(wvT_ref[...], x).astype(bf16)
    w = lax.broadcasted_iota(jnp.int32, (3 * BQ, BQ), 0)
    qi = lax.broadcasted_iota(jnp.int32, (3 * BQ, BQ), 1)
    rel = qi + 256 - w
    valid = (rel >= 0) & (rel < W) & (w + (i - 2) * BQ >= 0)
    bias_s[...] = jnp.where(valid, 0.0, -1e9).astype(f32)

    def qk(hg, dst):
        g = hg // 2
        c0 = pl.multiple_of((hg % 2) * 512, 512)
        kw = kc_s[g, pl.ds(pl.multiple_of(i * BQ, BQ), 3 * BQ), :]
        s = _dot(kw, qm_s[g, :, pl.ds(c0, 512)])
        b = bias_s[...]
        for hh in range(4):
            dst[:, hh * 128:(hh + 1) * 128] = s[:, hh * 128:(hh + 1) * 128] + b

    def softmax_pv(hg, src):
        s = src[...]
        m = jnp.max(s, axis=0, keepdims=True)
        p = jnp.exp(s - m)
        l = jnp.sum(p, axis=0, keepdims=True)
        pb = p.astype(bf16)
        rl = 1.0 / l
        for hh in range(4):
            r0 = pl.multiple_of((hg * 4 + hh) * 16, 16)
            cs = slice(hh * 128, (hh + 1) * 128)
            o = _dot(vc_s[i, pl.ds(r0, 16), :], pb[0:128, cs])
            o = o + _dot(vc_s[i + 1, pl.ds(r0, 16), :], pb[128:256, cs])
            o = o + _dot(vc_s[i + 2, pl.ds(r0, 16), :], pb[256:384, cs])
            ot_s[pl.ds(r0, 16), :] = (o * rl[:, cs]).astype(bf16)

    qk(0, sa_s)

    def hbody_a(t, carry):
        hg = 2 * t
        qk(hg + 1, sb_s)
        softmax_pv(hg, sa_s)
        qk(hg + 2, sa_s)
        softmax_pv(hg + 1, sb_s)
        return carry
    lax.fori_loop(0, 3, hbody_a, 0)
    qk(7, sb_s)
    softmax_pv(6, sa_s)
    softmax_pv(7, sb_s)

    out_a = lax.dot_general(ot_s[...], wo_ref[...], (((0,), (0,)), ((), ())), preferred_element_type=f32)
    o_ref[:, 0:D] = out_a.astype(bf16)

    DIRECT = (0, 3, 7)

    @pl.when(i == 0)
    def _prologue():
        dt = jnp.exp(ldt_ref[...].astype(f32)).astype(bf16).astype(f32)
        are = p_ref[0].astype(f32) * dt
        aim = p_ref[1].astype(f32) * dt
        bre = p_ref[2].astype(f32) * dt
        bim = p_ref[3].astype(f32) * dt
        cr, ci = _cmul(p_ref[4].astype(f32), p_ref[5].astype(f32), bre, bim)
        c_s[0] = cr
        c_s[1] = ci
        a_s[0] = cr
        a_s[1] = ci
        uh_s[0] = jnp.zeros((2 * T, D), f32)
        ap_s[...] = jnp.zeros(ap_s.shape, f32)
        for c in range(NC):
            kp_s[c] = jnp.zeros((2 * T, D), f32)
        for kk in range(11):
            if kk in DIRECT:
                s = float(2 ** kk)
                e = jnp.exp(are * s)
                th = aim * s
                pw_s[kk, 0] = e * jnp.cos(th)
                pw_s[kk, 1] = e * jnp.sin(th)
            else:
                pr, pi_ = pw_s[kk - 1, 0], pw_s[kk - 1, 1]
                pw_s[kk, 0] = pr * pr - pi_ * pi_
                pw_s[kk, 1] = 2.0 * (pr * pi_)

    reg = (i >= 2).astype(jnp.int32) + (i >= 4).astype(jnp.int32) + (i >= 8).astype(jnp.int32)

    for rg, start in enumerate([0, 2, 4, 8]):
        @pl.when(i == start)
        def _lo():
            e1r, e1i = pw_s[rg, 0], pw_s[rg, 1]
            e2r, e2i = pw_s[rg + 1, 0], pw_s[rg + 1, 1]
            e4r, e4i = pw_s[rg + 2, 0], pw_s[rg + 2, 1]
            lo_s[1, 0] = e1r; lo_s[1, 1] = e1i
            lo_s[2, 0] = e2r; lo_s[2, 1] = e2i
            e3r, e3i = _cmul(e1r, e1i, e2r, e2i)
            lo_s[3, 0] = e3r; lo_s[3, 1] = e3i
            lo_s[4, 0] = e4r; lo_s[4, 1] = e4i
            r, im = _cmul(e1r, e1i, e4r, e4i); lo_s[5, 0] = r; lo_s[5, 1] = im
            r, im = _cmul(e2r, e2i, e4r, e4i); lo_s[6, 0] = r; lo_s[6, 1] = im
            r, im = _cmul(e3r, e3i, e4r, e4i); lo_s[7, 0] = r; lo_s[7, 1] = im

    gr0, gi0 = a_s[0], a_s[1]
    g_s[0] = gr0
    g_s[1] = gi0
    nr0, ni0 = _cmul(gr0, gi0, pw_s[7, 0], pw_s[7, 1])
    a_s[0] = nr0
    a_s[1] = ni0

    kq_s[...] = jnp.zeros(kq_s.shape, f32)
    nh = lax.shift_right_logical(jnp.int32(16), reg)
    stepk = 3 + reg

    def hbody(h, carry):
        for lg in range(4):
            sl = slice(lg * 128, (lg + 1) * 128)
            acc = [None] * 8
            for nv in range(16):
                rs = slice(nv * 8, nv * 8 + 8)
                gr = g_s[0, rs, sl]; gi = g_s[1, rs, sl]
                acc[0] = gr if nv == 0 else acc[0] + gr
                for j0 in range(1, 8):
                    xr = gr * lo_s[j0, 0, rs, sl] - gi * lo_s[j0, 1, rs, sl]
                    acc[j0] = xr if nv == 0 else acc[j0] + xr
                nr, ni = _cmul(gr, gi, pw_s[stepk, 0, rs, sl], pw_s[stepk, 1, rs, sl])
                g_s[0, rs, sl] = nr; g_s[1, rs, sl] = ni
            rows = [jnp.sum(a_, axis=0, keepdims=True) for a_ in acc]
            kq_s[pl.ds(pl.multiple_of(h * 8, 8), 8), sl] = jnp.concatenate(rows, axis=0)
        return carry
    lax.fori_loop(0, nh, hbody, 0)

    @pl.when(reg >= 1)
    def _bnd():
        kq_s[pl.ds(pl.multiple_of(nh * 8, 8), 8), :] = jnp.concatenate(
            [jnp.sum(g_s[0], axis=0, keepdims=True), jnp.zeros((7, D), f32)], axis=0)

    kc = kq_s[...]
    khi = kc.astype(bf16)
    klo = (kc - khi.astype(f32)).astype(bf16)
    Ft = F_ref[reg]
    a2 = _dot(Ft, khi)
    ah = a2[:256] + a2[256:] + _dot(Ft[:256], klo)
    sg = (1 - 2 * (lax.broadcasted_iota(jnp.int32, (T, 1), 0) & 1)).astype(f32)
    kp_s[i, :T] = ap_s[:T] + sg * ah[T:]
    kp_s[i, T:] = ap_s[T:] - sg * ah[:T]
    ap_s[...] = ah

    u2 = _dot(F_ref[0], u_ref[...])
    uh_s[i + 1] = u2[:256] + u2[256:]

    y_s[...] = jnp.zeros(y_s.shape, f32)

    def mbody(t, carry):
        d1 = 2 * t; d2 = 2 * t + 1
        for rb in range(16):
            for lg in range(4):
                rs = slice(rb * 8, rb * 8 + 8); ri = slice(T + rb * 8, T + rb * 8 + 8)
                cs = slice(lg * 128, (lg + 1) * 128)
                k1r = kp_s[d1, rs, cs]; k1i = kp_s[d1, ri, cs]
                u1r = uh_s[i + 1 - d1, rs, cs]; u1i = uh_s[i + 1 - d1, ri, cs]
                k2r = kp_s[d2, rs, cs]; k2i = kp_s[d2, ri, cs]
                u2r = uh_s[i + 1 - d2, rs, cs]; u2i = uh_s[i + 1 - d2, ri, cs]
                y_s[rs, cs] = y_s[rs, cs] + ((k1r * u1r - k1i * u1i) + (k2r * u2r - k2i * u2i))
                y_s[ri, cs] = y_s[ri, cs] + ((k1r * u1i + k1i * u1r) + (k2r * u2i + k2i * u2r))
        return carry
    lax.fori_loop(0, (i + 2) // 2, mbody, 0)

    Y = y_s[...]
    yhi = Y.astype(bf16)
    ylo = (Y - yhi.astype(f32)).astype(bf16)
    IFt = IF_ref[...]
    y2 = _dot(IFt, yhi)
    y = y2[:T] + y2[T:] + _dot(IFt[:T], ylo)
    ud = (u_ref[...].astype(f32) * dsk_ref[...].astype(f32)).astype(bf16).astype(f32)
    o_ref[:, D:2 * D] = (y.astype(bf16).astype(f32) + ud).astype(bf16)


@jax.jit
def pallas_concat_heads__sliding_block__ssm_conv_s4__prompt_kernel(
    A_x: jax.Array,
    A_wqkv: jax.Array,
    A_wo: jax.Array,
    B_u: jax.Array,
    B_A_re: jax.Array,
    B_A_im: jax.Array,
    B_B_re: jax.Array,
    B_B_im: jax.Array,
    B_C_re: jax.Array,
    B_C_im: jax.Array,
    B_log_dt: jax.Array,
    B_Dskip: jax.Array,
):
    Ftab, IFtab = _dft_tables()
    Ftab = jnp.asarray(Ftab)
    IFtab = jnp.asarray(IFtab)
    params = jnp.stack([B_A_re.T, B_A_im.T, B_B_re.T, B_B_im.T, B_C_re.T, B_C_im.T], 0)
    wqkvT = A_wqkv.T
    const = lambda *shape: pl.BlockSpec(shape, lambda i: (0,) * len(shape))
    out = pl.pallas_call(
        _kernel,
        grid=(NQ,),
        in_specs=[pl.BlockSpec((BQ, D), lambda i: (i, 0)),
                  pl.BlockSpec((D, D), lambda i: (0, 0)),
                  pl.BlockSpec((D, D), lambda i: (0, 1)),
                  pl.BlockSpec((D, D), lambda i: (2, 0)),
                  pl.BlockSpec((D, D), lambda i: (0, 0)),
                  pl.BlockSpec((T, D), lambda i: (i, 0)), const(6, N, D), const(1, D), const(1, D),
                  const(4, 512, 128), const(256, 256)],
        out_specs=pl.BlockSpec((BQ, 2 * D), lambda i: (i, 0)),
        out_shape=jax.ShapeDtypeStruct((S, 2 * D), bf16),
        scratch_shapes=[
            pltpu.VMEM((4, (NQ + 2) * BQ, 128), bf16),
            pltpu.VMEM((NQ + 2, D, BQ), bf16),
            pltpu.VMEM((4, 128, 1024), bf16),
            pltpu.VMEM((3 * BQ, BQ), f32),
            pltpu.VMEM((D, BQ), bf16),
            pltpu.VMEM((3 * BQ, 512), f32),
            pltpu.VMEM((3 * BQ, 512), f32),
            pltpu.VMEM((2, N, D), f32),
            pltpu.VMEM((2, N, D), f32),
            pltpu.VMEM((11, 2, N, D), f32),
            pltpu.VMEM((8, 2, N, D), f32),
            pltpu.VMEM((2, N, D), f32),
            pltpu.VMEM((T, D), f32),
            pltpu.VMEM((NC + 1, 2 * T, D), f32),
            pltpu.VMEM((NC, 2 * T, D), f32),
            pltpu.VMEM((2 * T, D), f32),
            pltpu.VMEM((2 * T, D), f32),
        ],
        compiler_params=pltpu.CompilerParams(dimension_semantics=("arbitrary",), vmem_limit_bytes=100 * 1024 * 1024),
        name="concat_attn_ssm",
    )(A_x.reshape(S, D), wqkvT, A_wqkv, wqkvT, A_wo, B_u.reshape(L, D), params,
      B_log_dt.reshape(1, D), B_Dskip.reshape(1, D), Ftab, IFtab)
    return out.reshape(1, S, 2 * D)
```

```python
import functools

import jax
import jax.numpy as jnp
import ml_dtypes
import numpy as np
from jax import lax
from jax.experimental import pallas as pl
from jax.experimental.pallas import tpu as pltpu

S, D, H, DH, W = 2048, 512, 32, 16, 256
BQ = 128
NQ = S // BQ
L, N, T = 2048, 128, 128
NC = L // T
f32, bf16, i32 = jnp.float32, jnp.bfloat16, jnp.int32
KROWS = 768
CFG = dict(np_proj=5, np_heads=(5, 4), np_out=2, chain=True, chain_heads=False)


def _split_hi_lo(m):
    hi = m.astype(np.float32).astype(ml_dtypes.bfloat16)
    lo = (m - hi.astype(np.float64)).astype(np.float32).astype(ml_dtypes.bfloat16)
    return hi, lo


def _dft_tables():
    f = np.arange(T)[:, None]
    j = np.arange(T)[None, :]
    th = 2 * np.pi * (f + 0.5) * j / (2 * T)
    F1 = np.concatenate([np.cos(th), -np.sin(th)], 0)
    tabs = []
    for reg, sigma in enumerate([1, 2, 4, 8]):
        base = 0 if reg == 0 else T * sigma
        m = base + np.arange(T)
        r = m.astype(np.float32).astype(ml_dtypes.bfloat16).astype(np.float64)
        idx = np.round((r - base) / sigma).astype(np.int64)
        Fp = np.zeros((2 * T, T))
        for jj in range(T):
            Fp[:, idx[jj]] += F1[:, jj]
        hi, lo = _split_hi_lo(Fp)
        tabs.append(np.concatenate([hi, lo], 0))
    Ftab = np.stack(tabs, 0)
    t = (np.arange(T) + T)[:, None]
    f2 = np.arange(T)[None, :]
    th2 = 2 * np.pi * (f2 + 0.5) * t / (2 * T)
    IF = np.concatenate([np.cos(th2), -np.sin(th2)], 1) / T
    hi, lo = _split_hi_lo(IF)
    IFtab = np.concatenate([hi, lo], 0)
    return Ftab, IFtab


def _cmul(ar, ai, br, bi):
    return ar * br - ai * bi, ar * bi + ai * br


def _dot(a, b):
    return jnp.dot(a, b, preferred_element_type=f32)


def _nt(a, b):
    return lax.dot_general(a, b, (((1,), (1,)), ((), ())), preferred_element_type=f32)


def _kernel(x_ref, wqkv_ref, wo_ref, u_ref,
            are_ref, aim_ref, bre_ref, bim_ref, cre_ref, cim_ref, ldt_ref, dsk_ref, F_ref, IF_ref,
            o_ref,
            wqT_s, wvT_s, kc_s, vc_s, qm_s, bias_s, ot_s, sa_s, sb_s, sc_s, ma_s, mb_s, mc_s,
            z_s, pw_s, lo_s, g_s, kall_s, uh_s, kp_s, ap_s, y_s):
    s_id = pl.program_id(0)
    NS = CFG["np_proj"] + 2 * CFG["np_heads"][0] + CFG["np_heads"][1] + CFG["np_out"]
    DIRECT = (0, 3, 5)

    @pl.when(s_id == 0)
    def _setup():
        kc_s[:, 0:256, :] = jnp.zeros((4, 256, 128), bf16)
        vc_s[0:2] = jnp.zeros((2, D, BQ), bf16)
        qm_s[...] = jnp.zeros(qm_s.shape, bf16)
        z_s[...] = jnp.zeros(z_s.shape, i32)
        kall_s[...] = jnp.zeros(kall_s.shape, f32)
        uh_s[0] = jnp.zeros((2 * T, D), f32)
        ap_s[...] = jnp.zeros(ap_s.shape, f32)
        for c in range(NC):
            kp_s[c] = jnp.zeros((2 * T, D), f32)
        eye = (lax.broadcasted_iota(i32, (128, 128), 0) == lax.broadcasted_iota(i32, (128, 128), 1)).astype(bf16)
        for a in range(4):
            for b in range(4):
                wqT_s[a * 128:(a + 1) * 128, b * 128:(b + 1) * 128] = _nt(
                    eye, wqkv_ref[b * 128:(b + 1) * 128, a * 128:(a + 1) * 128]).astype(bf16)
                wvT_s[a * 128:(a + 1) * 128, b * 128:(b + 1) * 128] = _nt(
                    eye, wqkv_ref[b * 128:(b + 1) * 128, 2 * D + a * 128:2 * D + (a + 1) * 128]).astype(bf16)
        tr = lambda r: _nt(eye, r[...])
        dt = jnp.exp(ldt_ref[...].astype(f32)).astype(bf16).astype(f32)
        are = tr(are_ref) * dt
        aim = tr(aim_ref) * dt
        cr, ci = _cmul(tr(cre_ref), tr(cim_ref), tr(bre_ref) * dt, tr(bim_ref) * dt)
        for lg in range(4):
            cs = slice(lg * 128, (lg + 1) * 128)
            g_s[lg, 0] = cr[:, cs]
            g_s[lg, 1] = ci[:, cs]
            for kk in range(7):
                if kk in DIRECT:
                    sc = float(2 ** kk)
                    e = jnp.exp(are[:, cs] * sc)
                    th = aim[:, cs] * sc
                    pw_s[kk, 0, lg] = e * jnp.cos(th)
                    pw_s[kk, 1, lg] = e * jnp.sin(th)
                else:
                    pr, pi_ = pw_s[kk - 1, 0, lg], pw_s[kk - 1, 1, lg]
                    pw_s[kk, 0, lg] = pr * pr - pi_ * pi_
                    pw_s[kk, 1, lg] = 2.0 * (pr * pi_)
            for rg in range(4):
                e1r, e1i = pw_s[rg, 0, lg], pw_s[rg, 1, lg]
                e2r, e2i = pw_s[rg + 1, 0, lg], pw_s[rg + 1, 1, lg]
                e4r, e4i = pw_s[rg + 2, 0, lg], pw_s[rg + 2, 1, lg]
                lo_s[rg, 0, 0, lg] = e1r; lo_s[rg, 0, 1, lg] = e1i
                lo_s[rg, 1, 0, lg] = e2r; lo_s[rg, 1, 1, lg] = e2i
                e3r, e3i = _cmul(e1r, e1i, e2r, e2i)
                lo_s[rg, 2, 0, lg] = e3r; lo_s[rg, 2, 1, lg] = e3i
                lo_s[rg, 3, 0, lg] = e4r; lo_s[rg, 3, 1, lg] = e4i
                r, im = _cmul(e1r, e1i, e4r, e4i); lo_s[rg, 4, 0, lg] = r; lo_s[rg, 4, 1, lg] = im
                r, im = _cmul(e2r, e2i, e4r, e4i); lo_s[rg, 5, 0, lg] = r; lo_s[rg, 5, 1, lg] = im
                r, im = _cmul(e3r, e3i, e4r, e4i); lo_s[rg, 6, 0, lg] = r; lo_s[rg, 6, 1, lg] = im

    sub = lax.broadcasted_iota(i32, (8, 128), 0)

    def kunits(base, n, chain=None):
        chain = CFG["chain"] if chain is None else chain
        if n == 0:
            return
        zm = z_s[...]
        tok = None
        for q in range(n):
            U = base + q
            Hh = U // 4
            lg = U % 4
            reg = (Hh >= 32).astype(i32) + (Hh >= 48).astype(i32) + (Hh >= 64).astype(i32)
            out = None
            for j0 in range(8):
                acc = None
                for nv in range(16):
                    rs = slice(nv * 8, nv * 8 + 8)
                    gr = g_s[lg, 0, rs, :]
                    if j0 == 0:
                        x = gr
                    else:
                        x = gr * lo_s[reg, j0 - 1, 0, lg, rs, :] - g_s[lg, 1, rs, :] * lo_s[reg, j0 - 1, 1, lg, rs, :]
                    if nv == 0:
                        acc = x if tok is None else x + tok
                    else:
                        acc = acc + x
                t_ = acc + pltpu.roll(acc, 4, 0)
                t_ = t_ + pltpu.roll(t_, 2, 0)
                t_ = t_ + pltpu.roll(t_, 1, 0)
                out = t_ if j0 == 0 else jnp.where(sub == j0, t_, out)
                if chain:
                    tok = lax.bitcast_convert_type(lax.bitcast_convert_type(t_, i32) & zm, f32)
            kall_s[pl.ds(pl.multiple_of(Hh * 8, 8), 8), pl.ds(pl.multiple_of(lg * 128, 128), 128)] = out
            for nv in range(16):
                rs = slice(nv * 8, nv * 8 + 8)
                nr, ni = _cmul(g_s[lg, 0, rs, :], g_s[lg, 1, rs, :],
                               pw_s[3 + reg, 0, lg, rs, :], pw_s[3 + reg, 1, lg, rs, :])
                g_s[lg, 0, rs, :] = nr
                g_s[lg, 1, rs, :] = ni

    @pl.when(s_id < NQ)
    def _phase_a():
        i = s_id
        ub = i * NS
        x = x_ref[...]
        k = _dot(x, wqkv_ref[:, D:2 * D]).astype(bf16)
        row0 = pl.multiple_of((i + 2) * BQ, BQ)
        for g in range(4):
            kc_s[g, pl.ds(row0, BQ), :] = k[:, g * 128:(g + 1) * 128]
        qT = (_nt(wqT_s[...], x) * (0.25 * 1.4426950408889634)).astype(bf16)
        for h in range(H):
            hp = h % 8
            qm_s[h // 8, hp * 16:hp * 16 + 16, hp * 128:(hp + 1) * 128] = qT[h * 16:(h + 1) * 16, :]
        vc_s[i + 2] = _nt(wvT_s[...], x).astype(bf16)
        w = lax.broadcasted_iota(i32, (3 * BQ, BQ), 0)
        qi = lax.broadcasted_iota(i32, (3 * BQ, BQ), 1)
        rel = qi + 256 - w
        valid = (rel >= 0) & (rel < W) & (w + (i - 2) * BQ >= 0)
        bias_s[...] = jnp.where(valid, 0.0, -1e9).astype(f32)
        kunits(ub, CFG["np_proj"])
        ub = ub + CFG["np_proj"]

        def qk(hg, dst, mdst):
            g = hg // 2
            c0 = pl.multiple_of((hg % 2) * 512, 512)
            kw = kc_s[g, pl.ds(pl.multiple_of(i * BQ, BQ), 3 * BQ), :]
            s = _dot(kw, qm_s[g, :, pl.ds(c0, 512)])
            b = bias_s[...]
            for hh in range(4):
                sb = s[:, hh * 128:(hh + 1) * 128] + b
                dst[:, hh * 128:(hh + 1) * 128] = sb
                parts = [sb[r * 8:(r + 1) * 8, :] for r in range(48)]
                while len(parts) > 1:
                    parts = [jnp.maximum(parts[a], parts[a + 1]) for a in range(0, len(parts) - 1, 2)] + ([parts[-1]] if len(parts) % 2 else [])
                mdst[:, hh * 128:(hh + 1) * 128] = jnp.max(parts[0], axis=0, keepdims=True)

        def softmax_pv(hg, src, msrc):
            for hh in range(4):
                r0 = pl.multiple_of((hg * 4 + hh) * 16, 16)
                cs = slice(hh * 128, (hh + 1) * 128)
                m = msrc[:, cs]
                o = None
                lsum = None
                for t in range(3):
                    p = jnp.exp2(src[t * 128:(t + 1) * 128, cs] - m)
                    parts = [p[r * 8:(r + 1) * 8, :] for r in range(16)]
                    while len(parts) > 1:
                        parts = [parts[a] + parts[a + 1] for a in range(0, len(parts), 2)]
                    lsum = parts[0] if lsum is None else lsum + parts[0]
                    d = _dot(vc_s[i + t, pl.ds(r0, 16), :], p.astype(bf16))
                    o = d if o is None else o + d
                l = jnp.sum(lsum, axis=0, keepdims=True)
                ot_s[pl.ds(r0, 16), :] = (o * (1.0 / l)).astype(bf16)

        bufs = [(sa_s, ma_s), (sb_s, mb_s), (sc_s, mc_s)]
        qk(0, *bufs[0])
        qk(1, *bufs[1])
        nh = CFG["np_heads"]

        def hbody(t, carry):
            for j in range(3):
                hgi = 3 * t + j
                qk(hgi + 2, *bufs[(j + 2) % 3])
                softmax_pv(hgi, *bufs[j])
            kunits(ub + t * nh[0], nh[0], CFG["chain_heads"])
            return carry
        lax.fori_loop(0, 2, hbody, 0)
        ub = ub + 2 * nh[0]
        softmax_pv(6, *bufs[0])
        softmax_pv(7, *bufs[1])
        kunits(ub, nh[1], CFG["chain_heads"])
        ub = ub + nh[1]

        out_a = lax.dot_general(ot_s[...], wo_ref[...], (((0,), (0,)), ((), ())), preferred_element_type=f32)
        o_ref[...] = out_a.astype(bf16)
        kunits(ub, CFG["np_out"])

    @pl.when(s_id >= NQ)
    def _phase_b():
        c = s_id - NQ
        reg = (c >= 2).astype(i32) + (c >= 4).astype(i32) + (c >= 8).astype(i32)
        row0 = jnp.where(c < 2, c * 128, jnp.where(c < 4, 256 + (c - 2) * 64,
                         jnp.where(c < 8, 384 + (c - 4) * 32, 512 + (c - 8) * 16)))
        kc = kall_s[pl.ds(pl.multiple_of(row0, 8), T), :]
        khi = kc.astype(bf16)
        klo = (kc - khi.astype(f32)).astype(bf16)
        Ft = F_ref[reg]
        a2 = _dot(Ft, khi)
        ah = a2[:256] + a2[256:] + _dot(Ft[:256], klo)
        sg = (1 - 2 * (lax.broadcasted_iota(i32, (T, 1), 0) & 1)).astype(f32)
        kp_s[c, :T] = ap_s[:T] + sg * ah[T:]
        kp_s[c, T:] = ap_s[T:] - sg * ah[:T]
        ap_s[...] = ah

        u2 = _dot(F_ref[0], u_ref[...])
        uh_s[c + 1] = u2[:256] + u2[256:]

        y_s[...] = jnp.zeros(y_s.shape, f32)

        def mbody(t, carry):
            d1 = 2 * t; d2 = 2 * t + 1
            for rb in range(16):
                for lg in range(4):
                    rs = slice(rb * 8, rb * 8 + 8); ri = slice(T + rb * 8, T + rb * 8 + 8)
                    cs = slice(lg * 128, (lg + 1) * 128)
                    k1r = kp_s[d1, rs, cs]; k1i = kp_s[d1, ri, cs]
                    u1r = uh_s[c + 1 - d1, rs, cs]; u1i = uh_s[c + 1 - d1, ri, cs]
                    k2r = kp_s[d2, rs, cs]; k2i = kp_s[d2, ri, cs]
                    u2r = uh_s[c + 1 - d2, rs, cs]; u2i = uh_s[c + 1 - d2, ri, cs]
                    y_s[rs, cs] = y_s[rs, cs] + ((k1r * u1r - k1i * u1i) + (k2r * u2r - k2i * u2i))
                    y_s[ri, cs] = y_s[ri, cs] + ((k1r * u1i + k1i * u1r) + (k2r * u2i + k2i * u2r))
            return carry
        lax.fori_loop(0, (c + 2) // 2, mbody, 0)

        Y = y_s[...]
        yhi = Y.astype(bf16)
        ylo = (Y - yhi.astype(f32)).astype(bf16)
        IFt = IF_ref[...]
        y2 = _dot(IFt, yhi)
        y = y2[:T] + y2[T:] + _dot(IFt[:T], ylo)
        ud = (u_ref[...].astype(f32) * dsk_ref[...].astype(f32)).astype(bf16).astype(f32)
        o_ref[...] = (y.astype(bf16).astype(f32) + ud).astype(bf16)


@jax.jit
def pallas_concat_heads__sliding_block__ssm_conv_s4__prompt_kernel(
    A_x: jax.Array,
    A_wqkv: jax.Array,
    A_wo: jax.Array,
    B_u: jax.Array,
    B_A_re: jax.Array,
    B_A_im: jax.Array,
    B_B_re: jax.Array,
    B_B_im: jax.Array,
    B_C_re: jax.Array,
    B_C_im: jax.Array,
    B_log_dt: jax.Array,
    B_Dskip: jax.Array,
):
    Ftab, IFtab = _dft_tables()
    Ftab = jnp.asarray(Ftab)
    IFtab = jnp.asarray(IFtab)
    const = lambda *shape: pl.BlockSpec(shape, lambda s: (0,) * len(shape))
    out = pl.pallas_call(
        _kernel,
        grid=(NQ + NC,),
        in_specs=[pl.BlockSpec((BQ, D), lambda s: (jnp.minimum(s, NQ - 1), 0)),
                  const(D, 3 * D), const(D, D),
                  pl.BlockSpec((T, D), lambda s: (jnp.maximum(s - NQ, 0), 0)),
                  const(D, N), const(D, N), const(D, N), const(D, N), const(D, N), const(D, N),
                  const(1, D), const(1, D), const(4, 512, 128), const(256, 256)],
        out_specs=pl.BlockSpec((BQ, D), lambda s: (jnp.where(s < NQ, s, s - NQ), jnp.where(s < NQ, 0, 1))),
        out_shape=jax.ShapeDtypeStruct((S, 2 * D), bf16),
        scratch_shapes=[
            pltpu.VMEM((D, D), bf16),
            pltpu.VMEM((D, D), bf16),
            pltpu.VMEM((4, (NQ + 2) * BQ, 128), bf16),
            pltpu.VMEM((NQ + 2, D, BQ), bf16),
            pltpu.VMEM((4, 128, 1024), bf16),
            pltpu.VMEM((3 * BQ, BQ), f32),
            pltpu.VMEM((D, BQ), bf16),
            pltpu.VMEM((3 * BQ, 512), f32),
            pltpu.VMEM((3 * BQ, 512), f32),
            pltpu.VMEM((3 * BQ, 512), f32),
            pltpu.VMEM((1, 512), f32),
            pltpu.VMEM((1, 512), f32),
            pltpu.VMEM((1, 512), f32),
            pltpu.VMEM((8, 128), i32),
            pltpu.VMEM((7, 2, 4, N, 128), f32),
            pltpu.VMEM((4, 7, 2, 4, N, 128), f32),
            pltpu.VMEM((4, 2, N, 128), f32),
            pltpu.VMEM((KROWS, D), f32),
            pltpu.VMEM((NC + 1, 2 * T, D), f32),
            pltpu.VMEM((NC, 2 * T, D), f32),
            pltpu.VMEM((2 * T, D), f32),
            pltpu.VMEM((2 * T, D), f32),
        ],
        compiler_params=pltpu.CompilerParams(dimension_semantics=("arbitrary",), vmem_limit_bytes=110 * 1024 * 1024),
        name="concat_attn_ssm",
    )(A_x.reshape(S, D), A_wqkv, A_wo, B_u.reshape(L, D), B_A_re, B_A_im, B_B_re, B_B_im, B_C_re, B_C_im,
      B_log_dt.reshape(1, D), B_Dskip.reshape(1, D), Ftab, IFtab)
    return out.reshape(1, S, 2 * D)
```

```python
import jax
import jax.numpy as jnp
import ml_dtypes
import numpy as np
from jax import lax
from jax.experimental import pallas as pl
from jax.experimental.pallas import tpu as pltpu

S, D, H, DH, W = 2048, 512, 32, 16, 256
BQ = 128
NQ = S // BQ
L, N, T = 2048, 128, 128
NC = L // T
f32, bf16, i32 = jnp.float32, jnp.bfloat16, jnp.int32
KROWS = 1024
CFG = dict(np_proj=6, nhb=1, np_out=3, np_free=1, nb1=6, nb2=4, chain=True, nacc=2)


def _split_hi_lo(m):
    hi = m.astype(np.float32).astype(ml_dtypes.bfloat16)
    lo = (m - hi.astype(np.float64)).astype(np.float32).astype(ml_dtypes.bfloat16)
    return hi, lo


def _dft_tables():
    f = np.arange(T)[:, None]
    j = np.arange(T)[None, :]
    th = 2 * np.pi * (f + 0.5) * j / (2 * T)
    F1 = np.concatenate([np.cos(th), -np.sin(th)], 0)
    tabs = []
    for reg, sigma in enumerate([1, 2, 4, 8]):
        base = 0 if reg == 0 else T * sigma
        m = base + np.arange(T)
        r = m.astype(np.float32).astype(ml_dtypes.bfloat16).astype(np.float64)
        idx = np.round((r - base) / sigma).astype(np.int64)
        Fp = np.zeros((2 * T, T))
        for jj in range(T):
            Fp[:, idx[jj]] += F1[:, jj]
        hi, lo = _split_hi_lo(Fp)
        tabs.append(np.concatenate([hi, lo], 0))
    Ftab = np.stack(tabs, 0)
    t = (np.arange(T) + T)[:, None]
    f2 = np.arange(T)[None, :]
    th2 = 2 * np.pi * (f2 + 0.5) * t / (2 * T)
    IF = np.concatenate([np.cos(th2), -np.sin(th2)], 1) / T
    hi, lo = _split_hi_lo(IF)
    IFtab = np.concatenate([hi, lo], 0)
    return Ftab, IFtab


def _cmul(ar, ai, br, bi):
    return ar * br - ai * bi, ar * bi + ai * br


def _dot(a, b):
    return jnp.dot(a, b, preferred_element_type=f32)


def _nt(a, b):
    return lax.dot_general(a, b, (((1,), (1,)), ((), ())), preferred_element_type=f32)


def _kernel(x_ref, wqkv_ref, wo_ref, u_ref,
            are_ref, aim_ref, bre_ref, bim_ref, cre_ref, cim_ref, ldt_ref, dsk_ref, F_ref, IF_ref,
            o_ref,
            wqT_s, wvT_s, kc_s, vc_s, qm_s, bias_s, ot_s, sa_s, sb_s, sc_s, ma_s, mb_s, mc_s,
            z_s, pw_s, lo_s, g_s, kall_s, uh_s, kp_s, ap_s, y_s):
    s_id = pl.program_id(0)
    NS = CFG["np_proj"] + 2 * CFG["nhb"] + CFG["np_out"] + CFG["np_free"]
    NSB = CFG["nb1"] + CFG["nb2"]
    DIRECT = (0, 3, 5)

    @pl.when(s_id == 0)
    def _setup():
        kc_s[:, 0:256, :] = jnp.zeros((4, 256, 128), bf16)
        vc_s[0:2] = jnp.zeros((2, D, BQ), bf16)
        qm_s[...] = jnp.zeros(qm_s.shape, bf16)
        z_s[...] = jnp.zeros(z_s.shape, i32)
        kall_s[...] = jnp.zeros(kall_s.shape, f32)
        uh_s[0] = jnp.zeros((2 * T, D), f32)
        ap_s[...] = jnp.zeros(ap_s.shape, f32)
        for c in range(NC):
            kp_s[c] = jnp.zeros((2 * T, D), f32)
        eye = (lax.broadcasted_iota(i32, (128, 128), 0) == lax.broadcasted_iota(i32, (128, 128), 1)).astype(bf16)
        for a in range(4):
            for b in range(4):
                wqT_s[a * 128:(a + 1) * 128, b * 128:(b + 1) * 128] = _nt(
                    eye, wqkv_ref[b * 128:(b + 1) * 128, a * 128:(a + 1) * 128]).astype(bf16)
                wvT_s[a * 128:(a + 1) * 128, b * 128:(b + 1) * 128] = _nt(
                    eye, wqkv_ref[b * 128:(b + 1) * 128, 2 * D + a * 128:2 * D + (a + 1) * 128]).astype(bf16)
        tr = lambda r: _nt(eye, r[...])
        dt = jnp.exp(ldt_ref[...].astype(f32)).astype(bf16).astype(f32)
        are = tr(are_ref) * dt
        aim = tr(aim_ref) * dt
        cr, ci = _cmul(tr(cre_ref), tr(cim_ref), tr(bre_ref) * dt, tr(bim_ref) * dt)
        for lg in range(4):
            cs = slice(lg * 128, (lg + 1) * 128)
            g_s[lg, 0] = cr[:, cs]
            g_s[lg, 1] = ci[:, cs]
            for kk in range(7):
                if kk in DIRECT:
                    sc = float(2 ** kk)
                    e = jnp.exp(are[:, cs] * sc)
                    th = aim[:, cs] * sc
                    pw_s[kk, 0, lg] = e * jnp.cos(th)
                    pw_s[kk, 1, lg] = e * jnp.sin(th)
                else:
                    pr, pi_ = pw_s[kk - 1, 0, lg], pw_s[kk - 1, 1, lg]
                    pw_s[kk, 0, lg] = pr * pr - pi_ * pi_
                    pw_s[kk, 1, lg] = 2.0 * (pr * pi_)
            for rg in range(4):
                e1r, e1i = pw_s[rg, 0, lg], pw_s[rg, 1, lg]
                e2r, e2i = pw_s[rg + 1, 0, lg], pw_s[rg + 1, 1, lg]
                e4r, e4i = pw_s[rg + 2, 0, lg], pw_s[rg + 2, 1, lg]
                lo_s[rg, 0, 0, lg] = e1r; lo_s[rg, 0, 1, lg] = e1i
                lo_s[rg, 1, 0, lg] = e2r; lo_s[rg, 1, 1, lg] = e2i
                e3r, e3i = _cmul(e1r, e1i, e2r, e2i)
                lo_s[rg, 2, 0, lg] = e3r; lo_s[rg, 2, 1, lg] = e3i
                lo_s[rg, 3, 0, lg] = e4r; lo_s[rg, 3, 1, lg] = e4i
                r, im = _cmul(e1r, e1i, e4r, e4i); lo_s[rg, 4, 0, lg] = r; lo_s[rg, 4, 1, lg] = im
                r, im = _cmul(e2r, e2i, e4r, e4i); lo_s[rg, 5, 0, lg] = r; lo_s[rg, 5, 1, lg] = im
                r, im = _cmul(e3r, e3i, e4r, e4i); lo_s[rg, 6, 0, lg] = r; lo_s[rg, 6, 1, lg] = im

    sub = lax.broadcasted_iota(i32, (8, 128), 0)

    def kunits(base, n, chain=None):
        chain = CFG["chain"] if chain is None else chain
        if n == 0:
            return
        zm = z_s[...]
        tok = None
        for q in range(n):
            U = base + q
            Hh = U // 4
            lg = U % 4
            reg = (Hh >= 32).astype(i32) + (Hh >= 48).astype(i32) + (Hh >= 64).astype(i32)
            out = None
            for j0 in range(8):
                accs = [None] * CFG["nacc"]
                for nv in range(16):
                    rs = slice(nv * 8, nv * 8 + 8)
                    gr = g_s[lg, 0, rs, :]
                    if j0 == 0:
                        x = gr
                    else:
                        x = gr * lo_s[reg, j0 - 1, 0, lg, rs, :] - g_s[lg, 1, rs, :] * lo_s[reg, j0 - 1, 1, lg, rs, :]
                    a_ = nv % CFG["nacc"]
                    if nv == 0:
                        accs[a_] = x if tok is None else x + tok
                    else:
                        accs[a_] = x if accs[a_] is None else accs[a_] + x
                acc = accs[0]
                for a_ in accs[1:]:
                    acc = acc + a_
                t_ = acc + pltpu.roll(acc, 4, 0)
                t_ = t_ + pltpu.roll(t_, 2, 0)
                t_ = t_ + pltpu.roll(t_, 1, 0)
                out = t_ if j0 == 0 else jnp.where(sub == j0, t_, out)
                if chain:
                    tok = lax.bitcast_convert_type(lax.bitcast_convert_type(t_, i32) & zm, f32)
            kall_s[pl.ds(pl.multiple_of(Hh * 8, 8), 8), pl.ds(pl.multiple_of(lg * 128, 128), 128)] = out
            for nv in range(16):
                rs = slice(nv * 8, nv * 8 + 8)
                nr, ni = _cmul(g_s[lg, 0, rs, :], g_s[lg, 1, rs, :],
                               pw_s[3 + reg, 0, lg, rs, :], pw_s[3 + reg, 1, lg, rs, :])
                g_s[lg, 0, rs, :] = nr
                g_s[lg, 1, rs, :] = ni

    @pl.when(s_id < NQ)
    def _phase_a():
        i = s_id
        ub = i * NS
        x = x_ref[...]
        k = _dot(x, wqkv_ref[:, D:2 * D]).astype(bf16)
        row0 = pl.multiple_of((i + 2) * BQ, BQ)
        for g in range(4):
            kc_s[g, pl.ds(row0, BQ), :] = k[:, g * 128:(g + 1) * 128]
        qT = (_nt(wqT_s[...], x) * (0.25 * 1.4426950408889634)).astype(bf16)
        for h in range(H):
            hp = h % 8
            qm_s[h // 8, hp * 16:hp * 16 + 16, hp * 128:(hp + 1) * 128] = qT[h * 16:(h + 1) * 16, :]
        vc_s[i + 2] = _nt(wvT_s[...], x).astype(bf16)
        w = lax.broadcasted_iota(i32, (3 * BQ, BQ), 0)
        qi = lax.broadcasted_iota(i32, (3 * BQ, BQ), 1)
        rel = qi + 256 - w
        valid = (rel >= 0) & (rel < W) & (w + (i - 2) * BQ >= 0)
        bias_s[...] = jnp.where(valid, 0.0, -1e9).astype(f32)
        kunits(ub, CFG["np_proj"])
        ub = ub + CFG["np_proj"]

        def qk(hg, dst, mdst):
            g = hg // 2
            c0 = pl.multiple_of((hg % 2) * 512, 512)
            kw = kc_s[g, pl.ds(pl.multiple_of(i * BQ, BQ), 3 * BQ), :]
            s = _dot(kw, qm_s[g, :, pl.ds(c0, 512)])
            b = bias_s[...]
            for hh in range(4):
                sb = s[:, hh * 128:(hh + 1) * 128] + b
                dst[:, hh * 128:(hh + 1) * 128] = sb
                parts = [sb[r * 8:(r + 1) * 8, :] for r in range(48)]
                while len(parts) > 1:
                    parts = [jnp.maximum(parts[a], parts[a + 1]) for a in range(0, len(parts) - 1, 2)] + ([parts[-1]] if len(parts) % 2 else [])
                mdst[:, hh * 128:(hh + 1) * 128] = jnp.max(parts[0], axis=0, keepdims=True)

        def softmax_pv(hg, src, msrc):
            for hh in range(4):
                r0 = pl.multiple_of((hg * 4 + hh) * 16, 16)
                cs = slice(hh * 128, (hh + 1) * 128)
                m = msrc[:, cs]
                o = None
                lsum = None
                for t in range(3):
                    p = jnp.exp2(src[t * 128:(t + 1) * 128, cs] - m)
                    parts = [p[r * 8:(r + 1) * 8, :] for r in range(16)]
                    while len(parts) > 1:
                        parts = [parts[a] + parts[a + 1] for a in range(0, len(parts), 2)]
                    lsum = parts[0] if lsum is None else lsum + parts[0]
                    d = _dot(vc_s[i + t, pl.ds(r0, 16), :], p.astype(bf16))
                    o = d if o is None else o + d
                l = jnp.sum(lsum, axis=0, keepdims=True)
                ot_s[pl.ds(r0, 16), :] = (o * (1.0 / l)).astype(bf16)

        bufs = [(sa_s, ma_s), (sb_s, mb_s), (sc_s, mc_s)]
        qk(0, *bufs[0])
        qk(1, *bufs[1])

        def hbody(t, carry):
            for j in range(3):
                hgi = 3 * t + j
                qk(hgi + 2, *bufs[(j + 2) % 3])
                softmax_pv(hgi, *bufs[j])
            kunits(ub + t * CFG["nhb"], CFG["nhb"])
            return carry
        lax.fori_loop(0, 2, hbody, 0)
        softmax_pv(6, *bufs[0])
        softmax_pv(7, *bufs[1])
        ub = ub + 2 * CFG["nhb"]

        out_a = lax.dot_general(ot_s[...], wo_ref[...], (((0,), (0,)), ((), ())), preferred_element_type=f32)
        o_ref[...] = out_a.astype(bf16)
        kunits(ub, CFG["np_out"])
        kunits(ub + CFG["np_out"], CFG["np_free"], False)

    @pl.when(s_id >= NQ)
    def _phase_b():
        c = s_id - NQ
        ubb = NQ * NS + c * NSB
        reg = (c >= 2).astype(i32) + (c >= 4).astype(i32) + (c >= 8).astype(i32)
        row0 = jnp.where(c < 2, c * 128, jnp.where(c < 4, 256 + (c - 2) * 64,
                         jnp.where(c < 8, 384 + (c - 4) * 32, 512 + (c - 8) * 16)))
        kc = kall_s[pl.ds(pl.multiple_of(row0, 8), T), :]
        khi = kc.astype(bf16)
        klo = (kc - khi.astype(f32)).astype(bf16)
        Ft = F_ref[reg]
        a2 = _dot(Ft, khi)
        ah = a2[:256] + a2[256:] + _dot(Ft[:256], klo)
        sg = (1 - 2 * (lax.broadcasted_iota(i32, (T, 1), 0) & 1)).astype(f32)
        kp_s[c, :T] = ap_s[:T] + sg * ah[T:]
        kp_s[c, T:] = ap_s[T:] - sg * ah[:T]
        ap_s[...] = ah

        u2 = _dot(F_ref[0], u_ref[...])
        uh_s[c + 1] = u2[:256] + u2[256:]
        kunits(ubb, CFG["nb1"])

        y_s[...] = jnp.zeros(y_s.shape, f32)

        def mbody(t, carry):
            d1 = 2 * t; d2 = 2 * t + 1
            for rb in range(16):
                for lg in range(4):
                    rs = slice(rb * 8, rb * 8 + 8); ri = slice(T + rb * 8, T + rb * 8 + 8)
                    cs = slice(lg * 128, (lg + 1) * 128)
                    k1r = kp_s[d1, rs, cs]; k1i = kp_s[d1, ri, cs]
                    u1r = uh_s[c + 1 - d1, rs, cs]; u1i = uh_s[c + 1 - d1, ri, cs]
                    k2r = kp_s[d2, rs, cs]; k2i = kp_s[d2, ri, cs]
                    u2r = uh_s[c + 1 - d2, rs, cs]; u2i = uh_s[c + 1 - d2, ri, cs]
                    y_s[rs, cs] = y_s[rs, cs] + ((k1r * u1r - k1i * u1i) + (k2r * u2r - k2i * u2i))
                    y_s[ri, cs] = y_s[ri, cs] + ((k1r * u1i + k1i * u1r) + (k2r * u2i + k2i * u2r))
            return carry
        lax.fori_loop(0, (c + 2) // 2, mbody, 0)

        Y = y_s[...]
        yhi = Y.astype(bf16)
        ylo = (Y - yhi.astype(f32)).astype(bf16)
        IFt = IF_ref[...]
        y2 = _dot(IFt, yhi)
        y = y2[:T] + y2[T:] + _dot(IFt[:T], ylo)
        ud = (u_ref[...].astype(f32) * dsk_ref[...].astype(f32)).astype(bf16).astype(f32)
        o_ref[...] = (y.astype(bf16).astype(f32) + ud).astype(bf16)
        kunits(ubb + CFG["nb1"], CFG["nb2"])


@jax.jit
def pallas_concat_heads__sliding_block__ssm_conv_s4__prompt_kernel(
    A_x: jax.Array,
    A_wqkv: jax.Array,
    A_wo: jax.Array,
    B_u: jax.Array,
    B_A_re: jax.Array,
    B_A_im: jax.Array,
    B_B_re: jax.Array,
    B_B_im: jax.Array,
    B_C_re: jax.Array,
    B_C_im: jax.Array,
    B_log_dt: jax.Array,
    B_Dskip: jax.Array,
):
    Ftab, IFtab = _dft_tables()
    Ftab = jnp.asarray(Ftab)
    IFtab = jnp.asarray(IFtab)
    const = lambda *shape: pl.BlockSpec(shape, lambda s: (0,) * len(shape))
    out = pl.pallas_call(
        _kernel,
        grid=(NQ + NC,),
        in_specs=[pl.BlockSpec((BQ, D), lambda s: (jnp.minimum(s, NQ - 1), 0)),
                  const(D, 3 * D), const(D, D),
                  pl.BlockSpec((T, D), lambda s: (jnp.maximum(s - NQ, 0), 0)),
                  const(D, N), const(D, N), const(D, N), const(D, N), const(D, N), const(D, N),
                  const(1, D), const(1, D), const(4, 512, 128), const(256, 256)],
        out_specs=pl.BlockSpec((BQ, D), lambda s: (jnp.where(s < NQ, s, s - NQ), jnp.where(s < NQ, 0, 1))),
        out_shape=jax.ShapeDtypeStruct((S, 2 * D), bf16),
        scratch_shapes=[
            pltpu.VMEM((D, D), bf16),
            pltpu.VMEM((D, D), bf16),
            pltpu.VMEM((4, (NQ + 2) * BQ, 128), bf16),
            pltpu.VMEM((NQ + 2, D, BQ), bf16),
            pltpu.VMEM((4, 128, 1024), bf16),
            pltpu.VMEM((3 * BQ, BQ), f32),
            pltpu.VMEM((D, BQ), bf16),
            pltpu.VMEM((3 * BQ, 512), f32),
            pltpu.VMEM((3 * BQ, 512), f32),
            pltpu.VMEM((3 * BQ, 512), f32),
            pltpu.VMEM((1, 512), f32),
            pltpu.VMEM((1, 512), f32),
            pltpu.VMEM((1, 512), f32),
            pltpu.VMEM((8, 128), i32),
            pltpu.VMEM((7, 2, 4, N, 128), f32),
            pltpu.VMEM((4, 7, 2, 4, N, 128), f32),
            pltpu.VMEM((4, 2, N, 128), f32),
            pltpu.VMEM((KROWS, D), f32),
            pltpu.VMEM((NC + 1, 2 * T, D), f32),
            pltpu.VMEM((NC, 2 * T, D), f32),
            pltpu.VMEM((2 * T, D), f32),
            pltpu.VMEM((2 * T, D), f32),
        ],
        compiler_params=pltpu.CompilerParams(dimension_semantics=("arbitrary",), vmem_limit_bytes=110 * 1024 * 1024),
        name="concat_attn_ssm",
    )(A_x.reshape(S, D), A_wqkv, A_wo, B_u.reshape(L, D), B_A_re, B_A_im, B_B_re, B_B_im, B_C_re, B_C_im,
      B_log_dt.reshape(1, D), B_Dskip.reshape(1, D), Ftab, IFtab)
    return out.reshape(1, S, 2 * D)
```

```python
import jax
import jax.numpy as jnp
import ml_dtypes
import numpy as np
from jax import lax
from jax.experimental import pallas as pl
from jax.experimental.pallas import tpu as pltpu

S, D, H, DH, W = 2048, 512, 32, 16, 256
BQ = 128
NQ = S // BQ
L, N, T = 2048, 128, 128
NC = L // T
f32, bf16, i32 = jnp.float32, jnp.bfloat16, jnp.int32
KROWS = 1024
CFG = dict(np_proj=6, nhb=1, np_out=3, np_free=1, nb1=6, nb2=4, chain=True, nacc=2)


def _split_hi_lo(m):
    hi = m.astype(np.float32).astype(ml_dtypes.bfloat16)
    lo = (m - hi.astype(np.float64)).astype(np.float32).astype(ml_dtypes.bfloat16)
    return hi, lo


def _dft_tables():
    f = np.arange(T)[:, None]
    j = np.arange(T)[None, :]
    th = 2 * np.pi * (f + 0.5) * j / (2 * T)
    F1 = np.concatenate([np.cos(th), -np.sin(th)], 0)
    tabs = []
    for reg, sigma in enumerate([1, 2, 4, 8]):
        base = 0 if reg == 0 else T * sigma
        m = base + np.arange(T)
        r = m.astype(np.float32).astype(ml_dtypes.bfloat16).astype(np.float64)
        idx = np.round((r - base) / sigma).astype(np.int64)
        Fp = np.zeros((2 * T, T))
        for jj in range(T):
            Fp[:, idx[jj]] += F1[:, jj]
        hi, lo = _split_hi_lo(Fp)
        tabs.append(np.concatenate([hi, lo], 0))
    Ftab = np.stack(tabs, 0)
    t = (np.arange(T) + T)[:, None]
    f2 = np.arange(T)[None, :]
    th2 = 2 * np.pi * (f2 + 0.5) * t / (2 * T)
    IF = np.concatenate([np.cos(th2), -np.sin(th2)], 1) / T
    hi, lo = _split_hi_lo(IF)
    IFtab = np.concatenate([hi, lo], 0)
    return Ftab, IFtab


def _check_schedule():
    n_a = CFG["np_proj"] + 2 * CFG["nhb"] + CFG["np_out"] + CFG["np_free"]
    n_b = CFG["nb1"] + CFG["nb2"]
    first_group = [0, 16, 32, 40, 48, 52, 56, 60] + [64 + 2 * k for k in range(8)] + [80]
    for c in range(NC):
        need = 4 * (first_group[c + 1] + (1 if c >= 2 else 0))
        assert need <= NQ * n_a + c * n_b, (c, need)
    assert 8 * ((NQ * n_a + NC * n_b - 1) // 4) + 8 <= KROWS


_check_schedule()


def _cmul(ar, ai, br, bi):
    return ar * br - ai * bi, ar * bi + ai * br


def _dot(a, b):
    return jnp.dot(a, b, preferred_element_type=f32)


def _nt(a, b):
    return lax.dot_general(a, b, (((1,), (1,)), ((), ())), preferred_element_type=f32)


def _sincos(th, small):
    def fast(th):
        k = jnp.round(th * 0.6366197723675814)
        r = th - k * 1.5703125
        r = r - k * 4.837512969970703125e-4
        r = r - k * 7.54978995489188216e-8
        r2 = r * r
        sn = r + r * r2 * (-1.6666654611e-1 + r2 * (8.3321608736e-3 + r2 * -1.9515295891e-4))
        cs = 1.0 - 0.5 * r2 + r2 * r2 * (4.166664568298827e-2 + r2 * (-1.388731625493765e-3 + r2 * 2.443315711809948e-5))
        ki = k.astype(i32)
        swap = (ki & 1) == 1
        s0 = jnp.where(swap, cs, sn)
        c0 = jnp.where(swap, sn, cs)
        return jnp.where((ki & 2) != 0, -s0, s0), jnp.where(((ki + 1) & 2) != 0, -c0, c0)

    def slow(th):
        return jnp.sin(th), jnp.cos(th)
    return lax.cond(small, fast, slow, th)


def _kernel(x_ref, wqkv_hbm, wo_hbm, u_ref,
            are_ref, aim_ref, bre_ref, bim_ref, cre_ref, cim_ref, ldt_ref, dsk_ref, F_hbm, IF_hbm,
            o_ref,
            wqkv_ref, wo_ref, F_ref, IF_ref, dma_sem, wqT_s, wvT_s, kc_s, vc_s, qm_s, bias_s, ot_s, sa_s, sb_s, sc_s, ma_s, mb_s, mc_s,
            z_s, pw_s, lo_s, g_s, kall_s, uh_s, kp_s, ap_s, y_s):
    s_id = pl.program_id(0)
    NS = CFG["np_proj"] + 2 * CFG["nhb"] + CFG["np_out"] + CFG["np_free"]
    NSB = CFG["nb1"] + CFG["nb2"]
    DIRECT = (0, 3, 5)

    @pl.when(s_id == 0)
    def _setup():
        copies = [pltpu.make_async_copy(src, dst, dma_sem.at[n])
                  for n, (src, dst) in enumerate([(wqkv_hbm, wqkv_ref), (wo_hbm, wo_ref), (F_hbm, F_ref), (IF_hbm, IF_ref)])]
        for cp in copies:
            cp.start()
        kc_s[:, 0:256, :] = jnp.zeros((4, 256, 128), bf16)
        vc_s[0:2] = jnp.zeros((2, D, BQ), bf16)
        qm_s[...] = jnp.zeros(qm_s.shape, bf16)
        z_s[...] = jnp.zeros(z_s.shape, i32)
        kall_s[...] = jnp.zeros(kall_s.shape, f32)
        uh_s[0] = jnp.zeros((2 * T, D), f32)
        ap_s[...] = jnp.zeros(ap_s.shape, f32)
        for c in range(NC):
            kp_s[c] = jnp.zeros((2 * T, D), f32)
        eye = (lax.broadcasted_iota(i32, (128, 128), 0) == lax.broadcasted_iota(i32, (128, 128), 1)).astype(bf16)
        tr = lambda r: _nt(eye, r[...])
        dt = jnp.exp(ldt_ref[...].astype(f32)).astype(bf16).astype(f32)
        are = tr(are_ref) * dt
        aim = tr(aim_ref) * dt
        cr, ci = _cmul(tr(cre_ref), tr(cim_ref), tr(bre_ref) * dt, tr(bim_ref) * dt)
        small = jnp.max(jnp.abs(aim)) * float(2 ** max(DIRECT)) < 8000.0
        for lg in range(4):
            cs = slice(lg * 128, (lg + 1) * 128)
            g_s[lg, 0] = cr[:, cs]
            g_s[lg, 1] = ci[:, cs]
            for kk in range(7):
                if kk in DIRECT:
                    sc = float(2 ** kk)
                    e = jnp.exp(are[:, cs] * sc)
                    th = aim[:, cs] * sc
                    sn, cs_ = _sincos(th, small)
                    pw_s[kk, 0, lg] = e * cs_
                    pw_s[kk, 1, lg] = e * sn
                else:
                    pr, pi_ = pw_s[kk - 1, 0, lg], pw_s[kk - 1, 1, lg]
                    pw_s[kk, 0, lg] = pr * pr - pi_ * pi_
                    pw_s[kk, 1, lg] = 2.0 * (pr * pi_)
            for rg in range(4):
                e1r, e1i = pw_s[rg, 0, lg], pw_s[rg, 1, lg]
                e2r, e2i = pw_s[rg + 1, 0, lg], pw_s[rg + 1, 1, lg]
                e4r, e4i = pw_s[rg + 2, 0, lg], pw_s[rg + 2, 1, lg]
                lo_s[rg, 0, 0, lg] = e1r; lo_s[rg, 0, 1, lg] = e1i
                lo_s[rg, 1, 0, lg] = e2r; lo_s[rg, 1, 1, lg] = e2i
                e3r, e3i = _cmul(e1r, e1i, e2r, e2i)
                lo_s[rg, 2, 0, lg] = e3r; lo_s[rg, 2, 1, lg] = e3i
                lo_s[rg, 3, 0, lg] = e4r; lo_s[rg, 3, 1, lg] = e4i
                r, im = _cmul(e1r, e1i, e4r, e4i); lo_s[rg, 4, 0, lg] = r; lo_s[rg, 4, 1, lg] = im
                r, im = _cmul(e2r, e2i, e4r, e4i); lo_s[rg, 5, 0, lg] = r; lo_s[rg, 5, 1, lg] = im
                r, im = _cmul(e3r, e3i, e4r, e4i); lo_s[rg, 6, 0, lg] = r; lo_s[rg, 6, 1, lg] = im

        copies[0].wait()
        for a in range(4):
            for b in range(4):
                wqT_s[a * 128:(a + 1) * 128, b * 128:(b + 1) * 128] = _nt(
                    eye, wqkv_ref[b * 128:(b + 1) * 128, a * 128:(a + 1) * 128]).astype(bf16)
                wvT_s[a * 128:(a + 1) * 128, b * 128:(b + 1) * 128] = _nt(
                    eye, wqkv_ref[b * 128:(b + 1) * 128, 2 * D + a * 128:2 * D + (a + 1) * 128]).astype(bf16)
        for cp in copies[1:]:
            cp.wait()

    sub = lax.broadcasted_iota(i32, (8, 128), 0)

    def kunits(base, n, chain=None):
        chain = CFG["chain"] if chain is None else chain
        if n == 0:
            return
        zm = z_s[...]
        tok = None
        for q in range(n):
            U = base + q
            Hh = U // 4
            lg = U % 4
            reg = (Hh >= 32).astype(i32) + (Hh >= 48).astype(i32) + (Hh >= 64).astype(i32)
            out = None
            for j0 in range(8):
                accs = [None] * CFG["nacc"]
                for nv in range(16):
                    rs = slice(nv * 8, nv * 8 + 8)
                    gr = g_s[lg, 0, rs, :]
                    if j0 == 0:
                        x = gr
                    else:
                        x = gr * lo_s[reg, j0 - 1, 0, lg, rs, :] - g_s[lg, 1, rs, :] * lo_s[reg, j0 - 1, 1, lg, rs, :]
                    a_ = nv % CFG["nacc"]
                    if nv == 0:
                        accs[a_] = x if tok is None else x + tok
                    else:
                        accs[a_] = x if accs[a_] is None else accs[a_] + x
                acc = accs[0]
                for a_ in accs[1:]:
                    acc = acc + a_
                t_ = acc + pltpu.roll(acc, 4, 0)
                t_ = t_ + pltpu.roll(t_, 2, 0)
                t_ = t_ + pltpu.roll(t_, 1, 0)
                out = t_ if j0 == 0 else jnp.where(sub == j0, t_, out)
                if chain:
                    tok = lax.bitcast_convert_type(lax.bitcast_convert_type(t_, i32) & zm, f32)
            kall_s[pl.ds(pl.multiple_of(Hh * 8, 8), 8), pl.ds(pl.multiple_of(lg * 128, 128), 128)] = out
            for nv in range(16):
                rs = slice(nv * 8, nv * 8 + 8)
                nr, ni = _cmul(g_s[lg, 0, rs, :], g_s[lg, 1, rs, :],
                               pw_s[3 + reg, 0, lg, rs, :], pw_s[3 + reg, 1, lg, rs, :])
                g_s[lg, 0, rs, :] = nr
                g_s[lg, 1, rs, :] = ni

    @pl.when(s_id < NQ)
    def _phase_a():
        i = s_id
        ub = i * NS
        x = x_ref[...]
        k = _dot(x, wqkv_ref[:, D:2 * D]).astype(bf16)
        row0 = pl.multiple_of((i + 2) * BQ, BQ)
        for g in range(4):
            kc_s[g, pl.ds(row0, BQ), :] = k[:, g * 128:(g + 1) * 128]
        qT = (_nt(wqT_s[...], x) * (0.25 * 1.4426950408889634)).astype(bf16)
        for h in range(H):
            hp = h % 8
            qm_s[h // 8, hp * 16:hp * 16 + 16, hp * 128:(hp + 1) * 128] = qT[h * 16:(h + 1) * 16, :]
        vc_s[i + 2] = _nt(wvT_s[...], x).astype(bf16)
        w = lax.broadcasted_iota(i32, (3 * BQ, BQ), 0)
        qi = lax.broadcasted_iota(i32, (3 * BQ, BQ), 1)
        rel = qi + 256 - w
        valid = (rel >= 0) & (rel < W) & (w + (i - 2) * BQ >= 0)
        bias_s[...] = jnp.where(valid, 0.0, -1e9).astype(f32)
        kunits(ub, CFG["np_proj"])
        ub = ub + CFG["np_proj"]

        def qk(hg, dst, mdst):
            g = hg // 2
            c0 = pl.multiple_of((hg % 2) * 512, 512)
            kw = kc_s[g, pl.ds(pl.multiple_of(i * BQ, BQ), 3 * BQ), :]
            s = _dot(kw, qm_s[g, :, pl.ds(c0, 512)])
            b = bias_s[...]
            for hh in range(4):
                sb = s[:, hh * 128:(hh + 1) * 128] + b
                dst[:, hh * 128:(hh + 1) * 128] = sb
                parts = [sb[r * 8:(r + 1) * 8, :] for r in range(48)]
                while len(parts) > 1:
                    parts = [jnp.maximum(parts[a], parts[a + 1]) for a in range(0, len(parts) - 1, 2)] + ([parts[-1]] if len(parts) % 2 else [])
                mdst[:, hh * 128:(hh + 1) * 128] = jnp.max(parts[0], axis=0, keepdims=True)

        def softmax_pv(hg, src, msrc):
            for hh in range(4):
                r0 = pl.multiple_of((hg * 4 + hh) * 16, 16)
                cs = slice(hh * 128, (hh + 1) * 128)
                m = msrc[:, cs]
                o = None
                lsum = None
                for t in range(3):
                    p = jnp.exp2(src[t * 128:(t + 1) * 128, cs] - m)
                    parts = [p[r * 8:(r + 1) * 8, :] for r in range(16)]
                    while len(parts) > 1:
                        parts = [parts[a] + parts[a + 1] for a in range(0, len(parts), 2)]
                    lsum = parts[0] if lsum is None else lsum + parts[0]
                    d = _dot(vc_s[i + t, pl.ds(r0, 16), :], p.astype(bf16))
                    o = d if o is None else o + d
                l = jnp.sum(lsum, axis=0, keepdims=True)
                ot_s[pl.ds(r0, 16), :] = (o * (1.0 / l)).astype(bf16)

        bufs = [(sa_s, ma_s), (sb_s, mb_s), (sc_s, mc_s)]
        qk(0, *bufs[0])
        qk(1, *bufs[1])

        def hbody(t, carry):
            for j in range(3):
                hgi = 3 * t + j
                qk(hgi + 2, *bufs[(j + 2) % 3])
                softmax_pv(hgi, *bufs[j])
            kunits(ub + t * CFG["nhb"], CFG["nhb"])
            return carry
        lax.fori_loop(0, 2, hbody, 0)
        softmax_pv(6, *bufs[0])
        softmax_pv(7, *bufs[1])
        ub = ub + 2 * CFG["nhb"]

        out_a = lax.dot_general(ot_s[...], wo_ref[...], (((0,), (0,)), ((), ())), preferred_element_type=f32)
        o_ref[...] = out_a.astype(bf16)
        kunits(ub, CFG["np_out"])
        kunits(ub + CFG["np_out"], CFG["np_free"], False)

    @pl.when(s_id >= NQ)
    def _phase_b():
        c = s_id - NQ
        ubb = NQ * NS + c * NSB
        reg = (c >= 2).astype(i32) + (c >= 4).astype(i32) + (c >= 8).astype(i32)
        row0 = jnp.where(c < 2, c * 128, jnp.where(c < 4, 256 + (c - 2) * 64,
                         jnp.where(c < 8, 384 + (c - 4) * 32, 512 + (c - 8) * 16)))
        kc = kall_s[pl.ds(pl.multiple_of(row0, 8), T), :]
        khi = kc.astype(bf16)
        klo = (kc - khi.astype(f32)).astype(bf16)
        Ft = F_ref[reg]
        a2 = _dot(Ft, khi)
        ah = a2[:256] + a2[256:] + _dot(Ft[:256], klo)
        sg = (1 - 2 * (lax.broadcasted_iota(i32, (T, 1), 0) & 1)).astype(f32)
        kp_s[c, :T] = ap_s[:T] + sg * ah[T:]
        kp_s[c, T:] = ap_s[T:] - sg * ah[:T]
        ap_s[...] = ah

        u2 = _dot(F_ref[0], u_ref[...])
        uh_s[c + 1] = u2[:256] + u2[256:]
        kunits(ubb, CFG["nb1"])

        y_s[...] = jnp.zeros(y_s.shape, f32)

        def mbody(t, carry):
            d1 = 2 * t; d2 = 2 * t + 1
            for rb in range(16):
                for lg in range(4):
                    rs = slice(rb * 8, rb * 8 + 8); ri = slice(T + rb * 8, T + rb * 8 + 8)
                    cs = slice(lg * 128, (lg + 1) * 128)
                    k1r = kp_s[d1, rs, cs]; k1i = kp_s[d1, ri, cs]
                    u1r = uh_s[c + 1 - d1, rs, cs]; u1i = uh_s[c + 1 - d1, ri, cs]
                    k2r = kp_s[d2, rs, cs]; k2i = kp_s[d2, ri, cs]
                    u2r = uh_s[c + 1 - d2, rs, cs]; u2i = uh_s[c + 1 - d2, ri, cs]
                    y_s[rs, cs] = y_s[rs, cs] + ((k1r * u1r - k1i * u1i) + (k2r * u2r - k2i * u2i))
                    y_s[ri, cs] = y_s[ri, cs] + ((k1r * u1i + k1i * u1r) + (k2r * u2i + k2i * u2r))
            return carry
        lax.fori_loop(0, (c + 2) // 2, mbody, 0)

        Y = y_s[...]
        yhi = Y.astype(bf16)
        ylo = (Y - yhi.astype(f32)).astype(bf16)
        IFt = IF_ref[...]
        y2 = _dot(IFt, yhi)
        y = y2[:T] + y2[T:] + _dot(IFt[:T], ylo)
        ud = (u_ref[...].astype(f32) * dsk_ref[...].astype(f32)).astype(bf16).astype(f32)
        o_ref[...] = (y.astype(bf16).astype(f32) + ud).astype(bf16)
        kunits(ubb + CFG["nb1"], CFG["nb2"])


@jax.jit
def pallas_concat_heads__sliding_block__ssm_conv_s4__prompt_kernel(
    A_x: jax.Array,
    A_wqkv: jax.Array,
    A_wo: jax.Array,
    B_u: jax.Array,
    B_A_re: jax.Array,
    B_A_im: jax.Array,
    B_B_re: jax.Array,
    B_B_im: jax.Array,
    B_C_re: jax.Array,
    B_C_im: jax.Array,
    B_log_dt: jax.Array,
    B_Dskip: jax.Array,
):
    Ftab, IFtab = _dft_tables()
    Ftab = jnp.asarray(Ftab)
    IFtab = jnp.asarray(IFtab)
    const = lambda *shape: pl.BlockSpec(shape, lambda s: (0,) * len(shape))
    hbm = pl.BlockSpec(memory_space=pl.ANY)
    out = pl.pallas_call(
        _kernel,
        grid=(NQ + NC,),
        in_specs=[pl.BlockSpec((BQ, D), lambda s: (jnp.minimum(s, NQ - 1), 0)),
                  hbm, hbm,
                  pl.BlockSpec((T, D), lambda s: (jnp.maximum(s - NQ, 0), 0)),
                  const(D, N), const(D, N), const(D, N), const(D, N), const(D, N), const(D, N),
                  const(1, D), const(1, D), hbm, hbm],
        out_specs=pl.BlockSpec((BQ, D), lambda s: (jnp.where(s < NQ, s, s - NQ), jnp.where(s < NQ, 0, 1))),
        out_shape=jax.ShapeDtypeStruct((S, 2 * D), bf16),
        scratch_shapes=[
            pltpu.VMEM((D, 3 * D), bf16),
            pltpu.VMEM((D, D), bf16),
            pltpu.VMEM((4, 512, 128), bf16),
            pltpu.VMEM((256, 256), bf16),
            pltpu.SemaphoreType.DMA((4,)),
            pltpu.VMEM((D, D), bf16),
            pltpu.VMEM((D, D), bf16),
            pltpu.VMEM((4, (NQ + 2) * BQ, 128), bf16),
            pltpu.VMEM((NQ + 2, D, BQ), bf16),
            pltpu.VMEM((4, 128, 1024), bf16),
            pltpu.VMEM((3 * BQ, BQ), f32),
            pltpu.VMEM((D, BQ), bf16),
            pltpu.VMEM((3 * BQ, 512), f32),
            pltpu.VMEM((3 * BQ, 512), f32),
            pltpu.VMEM((3 * BQ, 512), f32),
            pltpu.VMEM((1, 512), f32),
            pltpu.VMEM((1, 512), f32),
            pltpu.VMEM((1, 512), f32),
            pltpu.VMEM((8, 128), i32),
            pltpu.VMEM((7, 2, 4, N, 128), f32),
            pltpu.VMEM((4, 7, 2, 4, N, 128), f32),
            pltpu.VMEM((4, 2, N, 128), f32),
            pltpu.VMEM((KROWS, D), f32),
            pltpu.VMEM((NC + 1, 2 * T, D), f32),
            pltpu.VMEM((NC, 2 * T, D), f32),
            pltpu.VMEM((2 * T, D), f32),
            pltpu.VMEM((2 * T, D), f32),
        ],
        compiler_params=pltpu.CompilerParams(dimension_semantics=("arbitrary",), vmem_limit_bytes=110 * 1024 * 1024),
        name="concat_attn_ssm",
    )(A_x.reshape(S, D), A_wqkv, A_wo, B_u.reshape(L, D), B_A_re, B_A_im, B_B_re, B_B_im, B_C_re, B_C_im,
      B_log_dt.reshape(1, D), B_Dskip.reshape(1, D), Ftab, IFtab)
    return out.reshape(1, S, 2 * D)
```

```python
import jax
import jax.numpy as jnp
import ml_dtypes
import numpy as np
from jax import lax
from jax.experimental import pallas as pl
from jax.experimental.pallas import tpu as pltpu

S, D, H, DH, W = 2048, 512, 32, 16, 256
BQ = 128
NQ = S // BQ
L, N, T = 2048, 128, 128
NC = L // T
f32, bf16, i32 = jnp.float32, jnp.bfloat16, jnp.int32
KROWS = 768
CFG = dict(np_proj=12, nhb=1, np_out=3, np_free=0, nb1=2, nb2=3, chain=True, nacc=2)


def _split_hi_lo(m):
    hi = m.astype(np.float32).astype(ml_dtypes.bfloat16)
    lo = (m - hi.astype(np.float64)).astype(np.float32).astype(ml_dtypes.bfloat16)
    return hi, lo


def _dft_tables():
    f = np.arange(T)[:, None]
    j = np.arange(T)[None, :]
    th = 2 * np.pi * (f + 0.5) * j / (2 * T)
    F1 = np.concatenate([np.cos(th), -np.sin(th)], 0)
    tabs = []
    for reg, sigma in enumerate([1, 2, 4, 8]):
        base = 0 if reg == 0 else T * sigma
        m = base + np.arange(T)
        r = m.astype(np.float32).astype(ml_dtypes.bfloat16).astype(np.float64)
        idx = np.round((r - base) / sigma).astype(np.int64)
        Fp = np.zeros((2 * T, T))
        for jj in range(T):
            Fp[:, idx[jj]] += F1[:, jj]
        hi, lo = _split_hi_lo(Fp)
        tabs.append(np.concatenate([hi, lo], 0))
    Ftab = np.stack(tabs, 0)
    t = (np.arange(T) + T)[:, None]
    f2 = np.arange(T)[None, :]
    th2 = 2 * np.pi * (f2 + 0.5) * t / (2 * T)
    IF = np.concatenate([np.cos(th2), -np.sin(th2)], 1) / T
    hi, lo = _split_hi_lo(IF)
    IFtab = np.concatenate([hi, lo], 0)
    return Ftab, IFtab


def _check_schedule():
    n_a = CFG["np_proj"] + 2 * CFG["nhb"] + CFG["np_out"] + CFG["np_free"]
    n_b = CFG["nb1"] + CFG["nb2"]
    first_group = [0, 16, 32, 40, 48, 52, 56, 60] + [64 + 2 * k for k in range(8)] + [80]
    for c in range(NC):
        need = 4 * (first_group[c + 1] + (1 if c >= 2 else 0))
        assert need <= NQ * n_a + c * n_b, (c, need)
    assert 8 * ((NQ * n_a + NC * n_b - 1) // 4) + 8 <= KROWS


_check_schedule()


def _cmul(ar, ai, br, bi):
    return ar * br - ai * bi, ar * bi + ai * br


def _dot(a, b):
    return jnp.dot(a, b, preferred_element_type=f32)


def _nt(a, b):
    return lax.dot_general(a, b, (((1,), (1,)), ((), ())), preferred_element_type=f32)


def _sincos(th, small):
    def fast(th):
        k = jnp.round(th * 0.6366197723675814)
        r = th - k * 1.5703125
        r = r - k * 4.837512969970703125e-4
        r = r - k * 7.54978995489188216e-8
        r2 = r * r
        sn = r + r * r2 * (-1.6666654611e-1 + r2 * (8.3321608736e-3 + r2 * -1.9515295891e-4))
        cs = 1.0 - 0.5 * r2 + r2 * r2 * (4.166664568298827e-2 + r2 * (-1.388731625493765e-3 + r2 * 2.443315711809948e-5))
        ki = k.astype(i32)
        swap = (ki & 1) == 1
        s0 = jnp.where(swap, cs, sn)
        c0 = jnp.where(swap, sn, cs)
        return jnp.where((ki & 2) != 0, -s0, s0), jnp.where(((ki + 1) & 2) != 0, -c0, c0)

    def slow(th):
        return jnp.sin(th), jnp.cos(th)
    return lax.cond(small, fast, slow, th)


def _kernel(x_ref, wqkv_hbm, wo_hbm, u_ref,
            are_ref, aim_ref, bre_ref, bim_ref, cre_ref, cim_ref, ldt_ref, dsk_ref, F_hbm, IF_hbm,
            o_ref,
            wqkv_ref, wo_ref, F_ref, IF_ref, dma_sem, wqT_s, wvT_s, kc_s, vc_s, qm_s, bias_s, ot_s, sa_s, sb_s, sc_s, ma_s, mb_s, mc_s,
            z_s, pw_s, lo_s, g_s, kall_s, uh_s, kp_s, ap_s, y_s):
    s_id = pl.program_id(0)
    NS = CFG["np_proj"] + 2 * CFG["nhb"] + CFG["np_out"] + CFG["np_free"]
    NSB = CFG["nb1"] + CFG["nb2"]
    DIRECT = (0, 3, 5)

    @pl.when(s_id == 0)
    def _setup():
        copies = [pltpu.make_async_copy(src, dst, dma_sem.at[n])
                  for n, (src, dst) in enumerate([(wqkv_hbm, wqkv_ref), (wo_hbm, wo_ref), (F_hbm, F_ref), (IF_hbm, IF_ref)])]
        for cp in copies:
            cp.start()
        kc_s[:, 0:256, :] = jnp.zeros((4, 256, 128), bf16)
        vc_s[0:2] = jnp.zeros((2, D, BQ), bf16)
        qm_s[...] = jnp.zeros(qm_s.shape, bf16)
        z_s[...] = jnp.zeros(z_s.shape, i32)
        kall_s[...] = jnp.zeros(kall_s.shape, f32)
        uh_s[0] = jnp.zeros((2 * T, D), f32)
        ap_s[...] = jnp.zeros(ap_s.shape, f32)
        eye = (lax.broadcasted_iota(i32, (128, 128), 0) == lax.broadcasted_iota(i32, (128, 128), 1)).astype(bf16)
        tr = lambda r: _nt(eye, r[...])
        dt = jnp.exp(ldt_ref[...].astype(f32)).astype(bf16).astype(f32)
        are = tr(are_ref) * dt
        aim = tr(aim_ref) * dt
        cr, ci = _cmul(tr(cre_ref), tr(cim_ref), tr(bre_ref) * dt, tr(bim_ref) * dt)
        small = jnp.max(jnp.abs(aim)) * float(2 ** max(DIRECT)) < 8000.0
        for lg in range(4):
            cs = slice(lg * 128, (lg + 1) * 128)
            g_s[lg, 0] = cr[:, cs]
            g_s[lg, 1] = ci[:, cs]
            for kk in range(7):
                if kk in DIRECT:
                    sc = float(2 ** kk)
                    e = jnp.exp(are[:, cs] * sc)
                    th = aim[:, cs] * sc
                    sn, cs_ = _sincos(th, small)
                    pw_s[kk, 0, lg] = e * cs_
                    pw_s[kk, 1, lg] = e * sn
                else:
                    pr, pi_ = pw_s[kk - 1, 0, lg], pw_s[kk - 1, 1, lg]
                    pw_s[kk, 0, lg] = pr * pr - pi_ * pi_
                    pw_s[kk, 1, lg] = 2.0 * (pr * pi_)
            for rg in range(4):
                e1r, e1i = pw_s[rg, 0, lg], pw_s[rg, 1, lg]
                e2r, e2i = pw_s[rg + 1, 0, lg], pw_s[rg + 1, 1, lg]
                e4r, e4i = pw_s[rg + 2, 0, lg], pw_s[rg + 2, 1, lg]
                lo_s[rg, 0, 0, lg] = e1r; lo_s[rg, 0, 1, lg] = e1i
                lo_s[rg, 1, 0, lg] = e2r; lo_s[rg, 1, 1, lg] = e2i
                e3r, e3i = _cmul(e1r, e1i, e2r, e2i)
                lo_s[rg, 2, 0, lg] = e3r; lo_s[rg, 2, 1, lg] = e3i
                lo_s[rg, 3, 0, lg] = e4r; lo_s[rg, 3, 1, lg] = e4i
                r, im = _cmul(e1r, e1i, e4r, e4i); lo_s[rg, 4, 0, lg] = r; lo_s[rg, 4, 1, lg] = im
                r, im = _cmul(e2r, e2i, e4r, e4i); lo_s[rg, 5, 0, lg] = r; lo_s[rg, 5, 1, lg] = im
                r, im = _cmul(e3r, e3i, e4r, e4i); lo_s[rg, 6, 0, lg] = r; lo_s[rg, 6, 1, lg] = im

        copies[0].wait()
        for a in range(4):
            for b in range(4):
                wqT_s[a * 128:(a + 1) * 128, b * 128:(b + 1) * 128] = _nt(
                    eye, wqkv_ref[b * 128:(b + 1) * 128, a * 128:(a + 1) * 128]).astype(bf16)
                wvT_s[a * 128:(a + 1) * 128, b * 128:(b + 1) * 128] = _nt(
                    eye, wqkv_ref[b * 128:(b + 1) * 128, 2 * D + a * 128:2 * D + (a + 1) * 128]).astype(bf16)
        for cp in copies[1:]:
            cp.wait()

    sub = lax.broadcasted_iota(i32, (8, 128), 0)

    def kunits(base, n, chain=None):
        chain = CFG["chain"] if chain is None else chain
        if n == 0:
            return
        zm = z_s[...]
        tok = None
        for q in range(n):
            U = base + q
            Hh = U // 4
            lg = U % 4
            reg = (Hh >= 32).astype(i32) + (Hh >= 48).astype(i32) + (Hh >= 64).astype(i32)
            out = None
            for j0 in range(8):
                accs = [None] * CFG["nacc"]
                for nv in range(16):
                    rs = slice(nv * 8, nv * 8 + 8)
                    gr = g_s[lg, 0, rs, :]
                    if j0 == 0:
                        x = gr
                    else:
                        x = gr * lo_s[reg, j0 - 1, 0, lg, rs, :] - g_s[lg, 1, rs, :] * lo_s[reg, j0 - 1, 1, lg, rs, :]
                    a_ = nv % CFG["nacc"]
                    if nv == 0:
                        accs[a_] = x if tok is None else x + tok
                    else:
                        accs[a_] = x if accs[a_] is None else accs[a_] + x
                acc = accs[0]
                for a_ in accs[1:]:
                    acc = acc + a_
                t_ = acc + pltpu.roll(acc, 4, 0)
                t_ = t_ + pltpu.roll(t_, 2, 0)
                t_ = t_ + pltpu.roll(t_, 1, 0)
                out = t_ if j0 == 0 else jnp.where(sub == j0, t_, out)
                if chain:
                    tok = lax.bitcast_convert_type(lax.bitcast_convert_type(t_, i32) & zm, f32)
            kall_s[pl.ds(pl.multiple_of(Hh * 8, 8), 8), pl.ds(pl.multiple_of(lg * 128, 128), 128)] = out
            for nv in range(16):
                rs = slice(nv * 8, nv * 8 + 8)
                nr, ni = _cmul(g_s[lg, 0, rs, :], g_s[lg, 1, rs, :],
                               pw_s[3 + reg, 0, lg, rs, :], pw_s[3 + reg, 1, lg, rs, :])
                g_s[lg, 0, rs, :] = nr
                g_s[lg, 1, rs, :] = ni

    @pl.when(s_id < NQ)
    def _phase_a():
        i = s_id
        ub = i * NS
        x = x_ref[...]
        k = _dot(x, wqkv_ref[:, D:2 * D]).astype(bf16)
        row0 = pl.multiple_of((i + 2) * BQ, BQ)
        for g in range(4):
            kc_s[g, pl.ds(row0, BQ), :] = k[:, g * 128:(g + 1) * 128]
        qT = (_nt(wqT_s[...], x) * (0.25 * 1.4426950408889634)).astype(bf16)
        for h in range(H):
            hp = h % 8
            qm_s[h // 8, hp * 16:hp * 16 + 16, hp * 128:(hp + 1) * 128] = qT[h * 16:(h + 1) * 16, :]
        vc_s[i + 2] = _nt(wvT_s[...], x).astype(bf16)
        w = lax.broadcasted_iota(i32, (3 * BQ, BQ), 0)
        qi = lax.broadcasted_iota(i32, (3 * BQ, BQ), 1)
        rel = qi + 256 - w
        valid = (rel >= 0) & (rel < W) & (w + (i - 2) * BQ >= 0)
        bias_s[...] = jnp.where(valid, 0.0, -1e9).astype(f32)
        u2 = _dot(F_ref[0], u_ref[...])
        uh_s[i + 1] = u2[:256] + u2[256:]
        kunits(ub, CFG["np_proj"])
        ub = ub + CFG["np_proj"]

        def qk(hg, dst, mdst):
            g = hg // 2
            c0 = pl.multiple_of((hg % 2) * 512, 512)
            kw = kc_s[g, pl.ds(pl.multiple_of(i * BQ, BQ), 3 * BQ), :]
            s = _dot(kw, qm_s[g, :, pl.ds(c0, 512)])
            b = bias_s[...]
            for hh in range(4):
                sb = s[:, hh * 128:(hh + 1) * 128] + b
                dst[:, hh * 128:(hh + 1) * 128] = sb
                parts = [sb[r * 8:(r + 1) * 8, :] for r in range(48)]
                while len(parts) > 1:
                    parts = [jnp.maximum(parts[a], parts[a + 1]) for a in range(0, len(parts) - 1, 2)] + ([parts[-1]] if len(parts) % 2 else [])
                mdst[:, hh * 128:(hh + 1) * 128] = jnp.max(parts[0], axis=0, keepdims=True)

        def softmax_pv(hg, src, msrc):
            for hh in range(4):
                r0 = pl.multiple_of((hg * 4 + hh) * 16, 16)
                cs = slice(hh * 128, (hh + 1) * 128)
                m = msrc[:, cs]
                o = None
                lsum = None
                for t in range(3):
                    p = jnp.exp2(src[t * 128:(t + 1) * 128, cs] - m)
                    parts = [p[r * 8:(r + 1) * 8, :] for r in range(16)]
                    while len(parts) > 1:
                        parts = [parts[a] + parts[a + 1] for a in range(0, len(parts), 2)]
                    lsum = parts[0] if lsum is None else lsum + parts[0]
                    d = _dot(vc_s[i + t, pl.ds(r0, 16), :], p.astype(bf16))
                    o = d if o is None else o + d
                l = jnp.sum(lsum, axis=0, keepdims=True)
                ot_s[pl.ds(r0, 16), :] = (o * (1.0 / l)).astype(bf16)

        bufs = [(sa_s, ma_s), (sb_s, mb_s), (sc_s, mc_s)]
        qk(0, *bufs[0])
        qk(1, *bufs[1])

        def hbody(t, carry):
            for j in range(3):
                hgi = 3 * t + j
                qk(hgi + 2, *bufs[(j + 2) % 3])
                softmax_pv(hgi, *bufs[j])
            kunits(ub + t * CFG["nhb"], CFG["nhb"])
            return carry
        lax.fori_loop(0, 2, hbody, 0)
        softmax_pv(6, *bufs[0])
        softmax_pv(7, *bufs[1])
        ub = ub + 2 * CFG["nhb"]

        out_a = lax.dot_general(ot_s[...], wo_ref[...], (((0,), (0,)), ((), ())), preferred_element_type=f32)
        o_ref[...] = out_a.astype(bf16)
        kunits(ub, CFG["np_out"])
        kunits(ub + CFG["np_out"], CFG["np_free"], False)

    @pl.when(s_id >= NQ)
    def _phase_b():
        c = s_id - NQ
        ubb = NQ * NS + c * NSB
        reg = (c >= 2).astype(i32) + (c >= 4).astype(i32) + (c >= 8).astype(i32)
        row0 = jnp.where(c < 2, c * 128, jnp.where(c < 4, 256 + (c - 2) * 64,
                         jnp.where(c < 8, 384 + (c - 4) * 32, 512 + (c - 8) * 16)))
        kc = kall_s[pl.ds(pl.multiple_of(row0, 8), T), :]
        khi = kc.astype(bf16)
        klo = (kc - khi.astype(f32)).astype(bf16)
        Ft = F_ref[reg]
        a2 = _dot(Ft, khi)
        ah = a2[:256] + a2[256:] + _dot(Ft[:256], klo)
        sg = (1 - 2 * (lax.broadcasted_iota(i32, (T, 1), 0) & 1)).astype(f32)
        kp_s[c, :T] = ap_s[:T] + sg * ah[T:]
        kp_s[c, T:] = ap_s[T:] - sg * ah[:T]
        ap_s[...] = ah

        kunits(ubb, CFG["nb1"])

        y_s[...] = jnp.zeros(y_s.shape, f32)

        def mbody(t, carry):
            d1 = 2 * t
            d2 = 2 * t + 1
            e2 = jnp.minimum(d2, c)
            for rb in range(16):
                for lg in range(4):
                    rs = slice(rb * 8, rb * 8 + 8); ri = slice(T + rb * 8, T + rb * 8 + 8)
                    cs = slice(lg * 128, (lg + 1) * 128)
                    k1r = kp_s[d1, rs, cs]; k1i = kp_s[d1, ri, cs]
                    u1r = uh_s[c + 1 - d1, rs, cs]; u1i = uh_s[c + 1 - d1, ri, cs]
                    k2r = kp_s[e2, rs, cs]; k2i = kp_s[e2, ri, cs]
                    u2r = uh_s[c + 1 - d2, rs, cs]; u2i = uh_s[c + 1 - d2, ri, cs]
                    y_s[rs, cs] = y_s[rs, cs] + ((k1r * u1r - k1i * u1i) + (k2r * u2r - k2i * u2i))
                    y_s[ri, cs] = y_s[ri, cs] + ((k1r * u1i + k1i * u1r) + (k2r * u2i + k2i * u2r))
            return carry
        lax.fori_loop(0, (c + 2) // 2, mbody, 0)

        Y = y_s[...]
        yhi = Y.astype(bf16)
        ylo = (Y - yhi.astype(f32)).astype(bf16)
        IFt = IF_ref[...]
        y2 = _dot(IFt, yhi)
        y = y2[:T] + y2[T:] + _dot(IFt[:T], ylo)
        ud = (u_ref[...].astype(f32) * dsk_ref[...].astype(f32)).astype(bf16).astype(f32)
        o_ref[...] = (y.astype(bf16).astype(f32) + ud).astype(bf16)
        kunits(ubb + CFG["nb1"], CFG["nb2"])


@jax.jit
def pallas_concat_heads__sliding_block__ssm_conv_s4__prompt_kernel(
    A_x: jax.Array,
    A_wqkv: jax.Array,
    A_wo: jax.Array,
    B_u: jax.Array,
    B_A_re: jax.Array,
    B_A_im: jax.Array,
    B_B_re: jax.Array,
    B_B_im: jax.Array,
    B_C_re: jax.Array,
    B_C_im: jax.Array,
    B_log_dt: jax.Array,
    B_Dskip: jax.Array,
):
    Ftab, IFtab = _dft_tables()
    Ftab = jnp.asarray(Ftab)
    IFtab = jnp.asarray(IFtab)
    const = lambda *shape: pl.BlockSpec(shape, lambda s: (0,) * len(shape))
    hbm = pl.BlockSpec(memory_space=pl.ANY)
    out = pl.pallas_call(
        _kernel,
        grid=(NQ + NC,),
        in_specs=[pl.BlockSpec((BQ, D), lambda s: (jnp.minimum(s, NQ - 1), 0)),
                  hbm, hbm,
                  pl.BlockSpec((T, D), lambda s: (jnp.where(s < NQ, s, s - NQ), 0)),
                  const(D, N), const(D, N), const(D, N), const(D, N), const(D, N), const(D, N),
                  const(1, D), const(1, D), hbm, hbm],
        out_specs=pl.BlockSpec((BQ, D), lambda s: (jnp.where(s < NQ, s, s - NQ), jnp.where(s < NQ, 0, 1))),
        out_shape=jax.ShapeDtypeStruct((S, 2 * D), bf16),
        scratch_shapes=[
            pltpu.VMEM((D, 3 * D), bf16),
            pltpu.VMEM((D, D), bf16),
            pltpu.VMEM((4, 512, 128), bf16),
            pltpu.VMEM((256, 256), bf16),
            pltpu.SemaphoreType.DMA((4,)),
            pltpu.VMEM((D, D), bf16),
            pltpu.VMEM((D, D), bf16),
            pltpu.VMEM((4, (NQ + 2) * BQ, 128), bf16),
            pltpu.VMEM((NQ + 2, D, BQ), bf16),
            pltpu.VMEM((4, 128, 1024), bf16),
            pltpu.VMEM((3 * BQ, BQ), f32),
            pltpu.VMEM((D, BQ), bf16),
            pltpu.VMEM((3 * BQ, 512), f32),
            pltpu.VMEM((3 * BQ, 512), f32),
            pltpu.VMEM((3 * BQ, 512), f32),
            pltpu.VMEM((1, 512), f32),
            pltpu.VMEM((1, 512), f32),
            pltpu.VMEM((1, 512), f32),
            pltpu.VMEM((8, 128), i32),
            pltpu.VMEM((7, 2, 4, N, 128), f32),
            pltpu.VMEM((4, 7, 2, 4, N, 128), f32),
            pltpu.VMEM((4, 2, N, 128), f32),
            pltpu.VMEM((KROWS, D), f32),
            pltpu.VMEM((NC + 1, 2 * T, D), f32),
            pltpu.VMEM((NC, 2 * T, D), f32),
            pltpu.VMEM((2 * T, D), f32),
            pltpu.VMEM((2 * T, D), f32),
        ],
        compiler_params=pltpu.CompilerParams(dimension_semantics=("arbitrary",), vmem_limit_bytes=110 * 1024 * 1024),
        name="concat_attn_ssm",
    )(A_x.reshape(S, D), A_wqkv, A_wo, B_u.reshape(L, D), B_A_re, B_A_im, B_B_re, B_B_im, B_C_re, B_C_im,
      B_log_dt.reshape(1, D), B_Dskip.reshape(1, D), Ftab, IFtab)
    return out.reshape(1, S, 2 * D)
```
